```python
import os as _os
_os.environ.setdefault("JAX_PLATFORMS", "cpu")
import jax
import jax.numpy as jnp

def _softmax(x, axis=-1):
    return jax.nn.softmax(x, axis=axis)
def _gelu(x):
    return jax.nn.gelu(x, approximate=True)
def _silu(x):
    return jax.nn.silu(x)
def _sigmoid(x):
    return jax.nn.sigmoid(x)
def _layernorm(x, axis=-1, eps=1e-5):
    m = jnp.mean(x, axis=axis, keepdims=True)
    v = jnp.var(x, axis=axis, keepdims=True)
    return (x - m) / jnp.sqrt(v + eps)
def _scatter_add(tgt, idx, src, axis=0):
    return tgt.at[idx].add(src)
def _segment_sum(src, seg, n):
    return jax.ops.segment_sum(src, seg, n)
class _Rng:
    def __init__(self, key):
        self._k = key
    def _next(self):
        self._k, sub = jax.random.split(self._k)
        return sub
    def normal(self, shape):
        return jax.random.normal(self._next(), shape, dtype=jnp.bfloat16)
    def randint(self, lo, hi, shape):
        return jax.random.randint(self._next(), shape, lo, hi, dtype=jnp.int32)
    def uniform(self, shape, lo=0.0, hi=1.0):
        return jax.random.uniform(self._next(), shape, jnp.bfloat16, lo, hi)
    def permutation(self, n):
        return jax.random.permutation(self._next(), n)


kernel_name = 'gated_mix__sliding_block_cached__swiglu_ffn__decode'

def setup_inputs():
    _rng = _Rng(jax.random.key(int.from_bytes(__import__("os").urandom(4), "little")))
    _w = (lambda a: (lambda t: t.astype(jnp.bfloat16) if jnp.issubdtype(t.dtype, jnp.floating) else t)(jnp.asarray(a)))
    def _A_setup():
        B, Sq, D = 1, 1, 512
        Hq, Hkv, Sk, Dh = 32, 32, 32768, 128
        assert Hq % Hkv == 0, (Hq, Hkv)
        return {
            "x": _w((lambda *s: _rng.normal(s) * 0.05)(B, Sq, D)),
            "k_cache": _w((lambda *s: _rng.normal(s) * 3.2)(B, Hkv, Sk, Dh)),
            "v_cache": _w((lambda *s: _rng.normal(s) * 1.6)(B, Hkv, Sk, Dh)),
            "wq": _w((lambda *s: _rng.normal(s) * 3.2)(D, Hq * Dh) * (D ** -0.5)),
            "wo": _w((lambda *s: _rng.normal(s) * 1.6)(Hq * Dh, D) * ((Hq * Dh) ** -0.5)),
        }
    _A_in = _A_setup()

    def _B_setup():
        B, S, D, F = 1, 1, 512, 1376
        return {
            "x": _w((lambda *s: _rng.normal(s) * 0.05)(B, S, D)),
            "w_gate": _w((lambda *s: _rng.normal(s) * 0.1)(D, F)),
            "w_up": _w((lambda *s: _rng.normal(s) * 0.1)(D, F)),
            "w_down": _w((lambda *s: _rng.normal(s) * 0.1)(F, D)),
        }
    _B_in = _B_setup()

    return {
        "A_x": _A_in["x"],
        "A_k_cache": _A_in["k_cache"],
        "A_v_cache": _A_in["v_cache"],
        "A_wq": _A_in["wq"],
        "A_wo": _A_in["wo"],
        "B_x": _B_in["x"],
        "B_w_gate": _B_in["w_gate"],
        "B_w_up": _B_in["w_up"],
        "B_w_down": _B_in["w_down"],
        "gate_w": _w((lambda *s: _rng.normal(s) * 0.05)(512) * 16.0),
    }

def reference(A_x, A_k_cache, A_v_cache, A_wq, A_wo, B_x, B_w_gate, B_w_up, B_w_down, gate_w):
    def _A_ref(x, k_cache, v_cache, wq, wo):
        B, Sq, D = x.shape
        Hq, Dh = 32, 128
        Hkv, Sk = k_cache.shape[1], k_cache.shape[2]
        W = min(4096, max(256, Sk // 4))
        rep = Hq // Hkv
        q = (lambda x, *d: x.transpose(*d))((x @ wq).reshape(B, Sq, Hq, Dh), 0, 2, 1, 3)
        k = jnp.repeat(k_cache[:, :, Sk - W:, :], rep, axis=1)
        v = jnp.repeat(v_cache[:, :, Sk - W:, :], rep, axis=1)
        scores = jnp.einsum("bhqd,bhkd->bhqk", q, k) * (Dh ** -0.5)
        p = _softmax(scores, axis=-1)
        o = jnp.einsum("bhqk,bhkd->bhqd", p, v)
        return (lambda x, *d: x.transpose(*d))(o, 0, 2, 1, 3).reshape(B, Sq, Hq * Dh) @ wo

    def _B_ref(x, w_gate, w_up, w_down):
        g = _silu(x @ w_gate)
        u = x @ w_up
        return (g * u) @ w_down

    x = A_x
    g = _sigmoid((x * gate_w).sum(-1, keepdims=True))
    a = _A_ref(x, A_k_cache, A_v_cache, A_wq, A_wo)
    b = _B_ref(x, B_w_gate, B_w_up, B_w_down)
    return g * a + (1 - g) * b
```

```python
import jax
import jax.numpy as jnp
from jax import lax
import jax.experimental.pallas as pl
import jax.experimental.pallas.tpu as pltpu

H, DH, D, F = 32, 128, 512, 1376
NT = (((1,), (1,)), ((), ()))


def _make_kernel(SK, W, depth=2):
    scale = DH ** -0.5

    def kernel(x_hbm, gw_hbm, k_hbm, v_hbm, wq_hbm, wo_hbm, wg_hbm, wu_hbm, wd_hbm, out_ref,
               xbuf, gwbuf, kbuf, vbuf, wqbuf, wobuf, wgbuf, wubuf, wdbuf, qscr, wsem, ksem, vsem):
        cx = pltpu.make_async_copy(x_hbm, xbuf, wsem.at[0])
        cgw = pltpu.make_async_copy(gw_hbm, gwbuf, wsem.at[1])
        cwq = pltpu.make_async_copy(wq_hbm, wqbuf, wsem.at[2])
        cwo = pltpu.make_async_copy(wo_hbm, wobuf, wsem.at[3])
        cwg = pltpu.make_async_copy(wg_hbm, wgbuf, wsem.at[4])
        cwu = pltpu.make_async_copy(wu_hbm, wubuf, wsem.at[5])
        cwd = pltpu.make_async_copy(wd_hbm, wdbuf, wsem.at[6])

        def ck(h):
            return pltpu.make_async_copy(k_hbm.at[0, h, pl.ds(SK - W, W), :], kbuf.at[h], ksem.at[h])

        def cv(h):
            return pltpu.make_async_copy(v_hbm.at[0, h, pl.ds(SK - W, W), :], vbuf.at[h], vsem.at[h])

        for c in (cx, cgw, cwq, cwo, cwg, cwu, cwd):
            c.start()
        for h in range(depth):
            ck(h).start()
            cv(h).start()

        cx.wait()
        cgw.wait()
        cwq.wait()
        x = xbuf[0]
        x8 = jnp.broadcast_to(x, (8, D))
        q = jnp.dot(x8, wqbuf[...], preferred_element_type=jnp.float32)
        qb = q.astype(jnp.bfloat16)
        for h in range(H):
            qscr[h] = qb[:, h * DH:(h + 1) * DH]

        cwo.wait()
        cwg.wait()
        cwu.wait()
        cwd.wait()
        g = lax.dot_general(x8, wgbuf[...], NT, preferred_element_type=jnp.float32)
        u = lax.dot_general(x8, wubuf[...], NT, preferred_element_type=jnp.float32)
        hh = (g * jax.nn.sigmoid(g) * u).astype(jnp.bfloat16)
        b = jnp.dot(hh, wdbuf[...], preferred_element_type=jnp.float32)

        def body(h, a):
            ck(h).wait()

            @pl.when(h + depth < H)
            def _():
                ck(h + depth).start()

            s = lax.dot_general(qscr[h], kbuf[h], NT, preferred_element_type=jnp.float32) * scale
            m = jnp.max(s, axis=-1, keepdims=True)
            p = jnp.exp(s - m)
            l = jnp.sum(p, axis=-1, keepdims=True)
            cv(h).wait()

            @pl.when(h + depth < H)
            def _():
                cv(h + depth).start()

            o = jnp.dot(p.astype(jnp.bfloat16), vbuf[h], preferred_element_type=jnp.float32) / l
            wo_h = wobuf[pl.ds(pl.multiple_of(h * DH, DH), DH), :]
            return a + jnp.dot(o.astype(jnp.bfloat16), wo_h, preferred_element_type=jnp.float32)

        a = lax.fori_loop(0, H, body, jnp.zeros((8, D), jnp.float32))

        xf = x.astype(jnp.float32)
        gw = gwbuf[...].astype(jnp.float32).reshape(1, D)
        gate = jax.nn.sigmoid(jnp.sum(xf * gw, axis=-1, keepdims=True))
        res = gate * a[0:1] + (1.0 - gate) * b[0:1]
        out_ref[0] = res.astype(out_ref.dtype)

    return kernel


@jax.jit
def pallas_gated_mix__sliding_block_cached__swiglu_ffn__decode_kernel(
    A_x: jax.Array,
    A_k_cache: jax.Array,
    A_v_cache: jax.Array,
    A_wq: jax.Array,
    A_wo: jax.Array,
    B_x: jax.Array,
    B_w_gate: jax.Array,
    B_w_up: jax.Array,
    B_w_down: jax.Array,
    gate_w: jax.Array,
):
    SK = A_k_cache.shape[2]
    W = min(4096, max(256, SK // 4))
    bf = jnp.bfloat16
    anyspec = pl.BlockSpec(memory_space=pl.ANY)
    return pl.pallas_call(
        _make_kernel(SK, W),
        out_shape=jax.ShapeDtypeStruct((1, 1, D), bf),
        in_specs=[anyspec] * 9,
        out_specs=pl.BlockSpec(memory_space=pltpu.VMEM),
        scratch_shapes=[
            pltpu.VMEM((1, 1, D), bf), pltpu.VMEM((D,), bf),
            pltpu.VMEM((H, W, DH), bf), pltpu.VMEM((H, W, DH), bf),
            pltpu.VMEM((D, H * DH), bf), pltpu.VMEM((H * DH, D), bf),
            pltpu.VMEM((F, D), bf), pltpu.VMEM((F, D), bf), pltpu.VMEM((F, D), bf),
            pltpu.VMEM((H, 8, DH), bf),
            pltpu.SemaphoreType.DMA((7,)), pltpu.SemaphoreType.DMA((H,)), pltpu.SemaphoreType.DMA((H,)),
        ],
        compiler_params=pltpu.CompilerParams(vmem_limit_bytes=110 * 1024 * 1024),
    )(A_x, gate_w, A_k_cache, A_v_cache, A_wq, A_wo, B_w_gate.T, B_w_up.T, B_w_down)
```

```python
import functools
import jax
import jax.numpy as jnp
from jax import lax
import jax.experimental.pallas as pl
import jax.experimental.pallas.tpu as pltpu

H, DH, D, F = 32, 128, 512, 1376
NT = (((1,), (1,)), ((), ()))
GH = 8
NG = H // GH
GW = GH * DH
ROWS = 128
WR = 32
QR = 16


def make_kernel(SK, W, nsub=4, dp=3, splits=(0, 1024, 1280, 1376), compute=True):
    scale = DH ** -0.5
    BK = ROWS * nsub
    PER = W // BK
    NB = dp + 1
    assert PER % NB == 0 and 2 <= dp < PER
    XO = (GW // WR) // PER
    XQ = (D // QR) // PER
    assert XO <= nsub and XQ <= nsub and XO * PER * WR == GW and XQ * PER * QR == D
    npiece = len(splits) - 1

    def kernel(x_hbm, gw_hbm, k_hbm, v_hbm, wq_hbm, wo_hbm, wg_hbm, wu_hbm, wd_hbm, out_ref,
               xbuf, gwbuf, ring, wqbuf, wobuf, wgbuf, wubuf, wdbuf, qscr, sscr, pscr, hscr,
               sem):
        XS, QS, OS, PS, DS = NB, NB + 1, NB + 2, NB + 3, NB + 4
        rsem = msem = sem

        def wait_on(ref, sem):
            pltpu.make_async_copy(ref, ref, sem).wait()

        def al(v, m):
            return v if isinstance(v, int) else pl.multiple_of(v, m)

        def wo_desc(g, i):
            r = al(i * WR, WR)
            return pltpu.make_async_copy(wo_hbm.at[pl.ds(al(g * GW + i * WR, WR), WR), :],
                                         wobuf.at[g, pl.ds(r, WR), :], msem.at[OS])

        def wq_desc(g, i):
            r = al(i * QR, QR)
            return pltpu.make_async_copy(wq_hbm.at[pl.ds(r, QR), pl.ds(al(g * GW, GW), GW)],
                                         wqbuf.at[pl.ds(r, QR), :], msem.at[QS])

        def issue(is_v, g, c):
            src = v_hbm if is_v else k_hbm
            slot = c % NB
            n = 0
            for sub in range(nsub):
                off = al(SK - W + c * BK + sub * ROWS, ROWS)
                for j in range(GH):
                    pltpu.make_async_copy(src.at[0, g * GH + j, pl.ds(off, ROWS), :],
                                          ring.at[slot, j, pl.ds(sub * ROWS, ROWS), :],
                                          rsem.at[slot]).start(priority=n % 2)
                    n += 1
                if not is_v and sub < XO:
                    wo_desc(g, c * XO + sub).start(priority=n % 2)
                    n += 1
                if is_v and sub < XQ:
                    pr = n % 2
                    @pl.when(g < NG - 1)
                    def _():
                        wq_desc(g + 1, c * XQ + sub).start(priority=pr)
                    n += 1

        def wd_issue(i):
            lo, hi = splits[i], splits[i + 1]
            nd = (hi - lo) // WR
            order = list(range(nd))
            if nd >= 16:
                half = nd // 2
                order = [x for pair in zip(range(half), range(half, nd)) for x in pair]
            for n, d in enumerate(order):
                r = lo + d * WR
                pltpu.make_async_copy(wd_hbm.at[pl.ds(r, WR), :], wdbuf.at[pl.ds(r, WR), :],
                                      msem.at[DS + i]).start(priority=n % 2)

        nw = F // WR
        descs = []
        streams = [[("q", i) for i in range(D // QR)],
                   [("g", i) for i in range(0, 22)], [("u", i) for i in range(0, 22)],
                   [("g", i) for i in range(22, nw)], [("u", i) for i in range(22, nw)]]
        tot = sum(len(s) for s in streams)
        keyed = []
        for si, s in enumerate(streams):
            for k, d in enumerate(s):
                keyed.append(((k + 0.5) / len(s), si, d))
        keyed.sort()
        for n, (_, _, (kind, i)) in enumerate(keyed):
            if kind == "q":
                wq_desc(0, i).start(priority=n % 2)
            else:
                src, dst = (wg_hbm, wgbuf) if kind == "g" else (wu_hbm, wubuf)
                pltpu.make_async_copy(src.at[pl.ds(i * WR, WR), :], dst.at[pl.ds(i * WR, WR), :],
                                      msem.at[PS]).start(priority=n % 2)
            if n == 0:
                pltpu.make_async_copy(x_hbm, xbuf, msem.at[XS]).start(priority=1)
                pltpu.make_async_copy(gw_hbm, gwbuf, msem.at[XS]).start(priority=0)
        tot_p = 2 * nw
        bounds = [round(tot_p * (i + 1) / dp) for i in range(dp)]
        prev = 0
        for i in range(dp):
            lo, hi = prev, bounds[i]
            prev = hi
            if lo < nw:
                e = min(hi, nw)
                wait_on(wgbuf.at[pl.ds(lo * WR, (e - lo) * WR), :], msem.at[PS])
            if hi > nw:
                s = max(lo, nw) - nw
                wait_on(wubuf.at[pl.ds(s * WR, (hi - nw - s) * WR), :], msem.at[PS])
            issue(False, 0, i)

        wait_on(xbuf, msem.at[XS])
        wait_on(gwbuf, msem.at[XS])
        x = xbuf[0]
        x8 = jnp.broadcast_to(x, (8, D))
        xf = x.astype(jnp.float32)
        gw = gwbuf[...].astype(jnp.float32).reshape(1, D)
        gate = jax.nn.sigmoid(jnp.sum(xf * gw, axis=-1, keepdims=True))
        gg = lax.dot_general(x8, wgbuf[...], NT, preferred_element_type=jnp.float32)
        uu = lax.dot_general(x8, wubuf[...], NT, preferred_element_type=jnp.float32)
        hscr[...] = (gg * jax.nn.sigmoid(gg) * uu).astype(jnp.bfloat16)

        row = lax.broadcasted_iota(jnp.int32, (GH, GW), 0)
        col = lax.broadcasted_iota(jnp.int32, (GH, GW), 1)
        diag = (col // DH) == row

        def group(g, a):
            wait_on(wqbuf, msem.at[QS])
            x8g = jnp.broadcast_to(xbuf[0], (8, D))
            q8 = jnp.dot(x8g, wqbuf[...], preferred_element_type=jnp.float32)
            qscr[...] = jnp.where(diag, q8, 0.0).astype(jnp.bfloat16)

            def kstep(c, carry):
                slot = c % NB
                wait_on(ring.at[slot], rsem.at[slot])
                @pl.when(c + dp < PER)
                def _():
                    issue(False, g, c + dp)
                @pl.when(c + dp >= PER)
                def _():
                    issue(True, g, c + dp - PER)
                s = None
                for j in range(GH):
                    t = lax.dot_general(qscr[:, j * DH:(j + 1) * DH], ring[slot, j], NT,
                                        preferred_element_type=jnp.float32)
                    s = t if s is None else s + t
                sscr[c] = s
                return carry
            lax.fori_loop(0, PER, kstep, 0)
            wait_on(wobuf.at[g], msem.at[OS])

            s = sscr[...] * scale
            m = jnp.max(jnp.max(s, axis=0), axis=-1, keepdims=True)
            p = jnp.exp(s - m[None])
            l = jnp.sum(jnp.sum(p, axis=0), axis=-1, keepdims=True)
            pscr[...] = p.astype(jnp.bfloat16)

            def vstep(c, o):
                slot = c % NB
                wait_on(ring.at[slot], rsem.at[slot])
                @pl.when(c + dp < PER)
                def _():
                    issue(True, g, c + dp)
                @pl.when(jnp.logical_and(c + dp >= PER, g < NG - 1))
                def _():
                    issue(False, g + 1, c + dp - PER)
                @pl.when(jnp.logical_and(c + dp == PER, g == NG - 1))
                def _():
                    wd_issue(0)
                @pl.when(jnp.logical_and(c + dp == PER + 1, g == NG - 1))
                def _():
                    for i in range(1, npiece):
                        wd_issue(i)
                pc = pscr[c]
                parts = [jnp.dot(pc, ring[slot, j], preferred_element_type=jnp.float32) for j in range(GH)]
                return o + jnp.concatenate(parts, axis=1)
            o = lax.fori_loop(0, PER, vstep, jnp.zeros((GH, GW), jnp.float32))
            ob = jnp.where(diag, o / l, 0.0).astype(jnp.bfloat16)
            return a + jnp.dot(ob, wobuf[g], preferred_element_type=jnp.float32)

        a = lax.fori_loop(0, NG, group, jnp.zeros((GH, D), jnp.float32))
        acc = gate * jnp.sum(a, axis=0, keepdims=True)
        omg = 1.0 - gate
        for i in range(npiece):
            lo, hi = splits[i], splits[i + 1]
            wait_on(wdbuf.at[pl.ds(lo, hi - lo), :], msem.at[DS + i])
            acc = acc + omg * jnp.dot(hscr[:, lo:hi], wdbuf[lo:hi, :], preferred_element_type=jnp.float32)[0:1]
        out_ref[0] = acc.astype(out_ref.dtype)
    return kernel


def build(dsc=True, dbc=True, **kw):
    nsub = kw.get("nsub", 4); dp = kw.get("dp", 3)
    npiece = len(kw.get("splits", (0, 1024, 1280, 1376))) - 1
    @jax.jit
    def fn(A_x, A_k_cache, A_v_cache, A_wq, A_wo, B_x, B_w_gate, B_w_up, B_w_down, gate_w):
        SK = A_k_cache.shape[2]
        W = min(4096, max(256, SK // 4))
        bf = jnp.bfloat16
        BK = ROWS * nsub
        PER = W // BK
        anyspec = pl.BlockSpec(memory_space=pl.ANY)
        return pl.pallas_call(
            make_kernel(SK, W, **kw),
            out_shape=jax.ShapeDtypeStruct((1, 1, D), bf),
            in_specs=[anyspec] * 9,
            out_specs=pl.BlockSpec(memory_space=pltpu.VMEM),
            scratch_shapes=[
                pltpu.VMEM((1, 1, D), bf), pltpu.VMEM((D,), bf),
                pltpu.VMEM((dp + 1, GH, BK, DH), bf),
                pltpu.VMEM((D, GW), bf), pltpu.VMEM((NG, GW, D), bf),
                pltpu.VMEM((F, D), bf), pltpu.VMEM((F, D), bf), pltpu.VMEM((F, D), bf),
                pltpu.VMEM((GH, GW), bf), pltpu.VMEM((PER, GH, BK), jnp.float32), pltpu.VMEM((PER, GH, BK), bf),
                pltpu.VMEM((8, F), bf),
                pltpu.SemaphoreType.DMA((dp + 1 + 4 + npiece,)),
            ],
            compiler_params=pltpu.CompilerParams(vmem_limit_bytes=64 * 1024 * 1024,
                                                 disable_semaphore_checks=dsc, disable_bounds_checks=dbc),
        )(A_x, gate_w, A_k_cache, A_v_cache, A_wq, A_wo, B_w_gate.T, B_w_up.T, B_w_down)
    return fn


_impl = build()


@jax.jit
def pallas_gated_mix__sliding_block_cached__swiglu_ffn__decode_kernel(
    A_x: jax.Array,
    A_k_cache: jax.Array,
    A_v_cache: jax.Array,
    A_wq: jax.Array,
    A_wo: jax.Array,
    B_x: jax.Array,
    B_w_gate: jax.Array,
    B_w_up: jax.Array,
    B_w_down: jax.Array,
    gate_w: jax.Array,
):
    return _impl(A_x, A_k_cache, A_v_cache, A_wq, A_wo, B_x, B_w_gate, B_w_up, B_w_down, gate_w)
```

```python
import jax
import jax.numpy as jnp
from jax import lax
import jax.experimental.pallas as pl
import jax.experimental.pallas.tpu as pltpu

H, DH, D, F = 32, 128, 512, 1376
NT = (((1,), (1,)), ((), ()))
GH = 8
NG = H // GH
GW = GH * DH
ROWS = 128
WR = 32


def _rr(streams):
    out = []
    for k in range(max(len(s) for s in streams)):
        for s in streams:
            if k < len(s):
                out.append(s[k])
    return out


def make_kernel(SK, W, nsub=4, dp=7, t0rows=640, splits=(0, 896, 1152, 1376), compute=True,
                ffn="C", porder="q,f"):
    scale = DH ** -0.5
    BK = ROWS * nsub
    PER = W // BK
    NB = dp + 1
    assert PER % NB == 0 and 2 <= dp < PER
    npiece = len(splits) - 1
    BATCH = GH * nsub
    NWO = 4

    def kernel(x_hbm, gw_hbm, k_hbm, v_hbm, wq_hbm, wo_hbm, wg_hbm, wu_hbm, wd_hbm, out_ref,
               xbuf, gwbuf, ring, wqbuf, wobuf, wgbuf, wubuf, wdbuf, qscr, sscr, pscr, hscr, oscr,
               sem):
        XS, QS, GS, US = NB, NB + 1, NB + 2, NB + 3
        OS = NB + 4
        DS = OS + NWO

        def wait_on(ref, s):
            pltpu.make_async_copy(ref, ref, sem.at[s]).wait()

        def al(v, m):
            return v if isinstance(v, int) else pl.multiple_of(v, m)

        def issue(is_v, g, c):
            src = v_hbm if is_v else k_hbm
            slot = c % NB
            n = 0
            for sub in range(nsub):
                off = al(SK - W + c * BK + sub * ROWS, ROWS)
                for j in range(GH):
                    pltpu.make_async_copy(src.at[0, g * GH + j, pl.ds(off, ROWS), :],
                                          ring.at[slot, j, pl.ds(sub * ROWS, ROWS), :],
                                          sem.at[slot]).start(priority=n % 2)
                    n += 1

        def rows_desc(src, dst, r, s):
            return pltpu.make_async_copy(src.at[pl.ds(r, WR), :], dst.at[pl.ds(r, WR), :], sem.at[s])

        def row_streams(lo, hi, stride):
            return [list(range(s, min(s + stride, hi), WR)) for s in range(lo, hi, stride)]

        def eissue(e):
            if e < NWO:
                n = 0
                for sub in range(DH // WR):
                    for j in range(8):
                        r = 512 * j + DH * e + WR * sub
                        pltpu.make_async_copy(wo_hbm.at[pl.ds(r, WR), :], wobuf.at[e, j, pl.ds(WR * sub, WR), :],
                                              sem.at[OS + e]).start(priority=n % 2)
                        n += 1
            elif e == NWO:
                t0 = list(range(0, t0rows, WR))
                t1 = list(range(t0rows, F, WR))
                def piece(r):
                    return max(i for i in range(npiece) if splits[i] <= r)
                seq = []
                for k in range(max(len(t0), len(t1))):
                    if k < len(t0): seq.append((t0[k], 0))
                    if k < len(t1): seq.append((t1[k], 1))
                for r, pr in seq:
                    rows_desc(wd_hbm, wdbuf, r, DS + piece(r)).start(priority=pr)
        NE = NWO + 1

        HQ = H * DH // 2
        wq_list = _rr([[("q", (64 * j + 8 * b, hh)) for b in range(8) for hh in range(2)] for j in range(8)])
        if ffn == "A":
            f_list = ([("g", r) for r in _rr(row_streams(0, F, 256))] + [("u", r) for r in _rr(row_streams(0, F, 256))])
        elif ffn == "B":
            f_list = _rr([[("g", r) for r in s] for s in row_streams(0, F, 512)] + [[("u", r) for r in s] for s in row_streams(0, F, 512)])
        elif ffn == "C":
            f_list = _rr([[("g", r) for r in s] for s in row_streams(0, F, 256)] + [[("u", r) for r in s] for s in row_streams(0, F, 256)])
        lists = dict(q=wq_list, f=f_list)
        plist = [d for k in porder.split(",") for d in lists[k]]

        def pdesc(d):
            kind, a = d
            if kind == "q":
                r, hh = a
                return pltpu.make_async_copy(wq_hbm.at[pl.ds(r, 8), pl.ds(hh * HQ, HQ)],
                                             wqbuf.at[pl.ds(r, 8), pl.ds(hh * HQ, HQ)], sem.at[QS])
            src, dst, s = dict(g=(wg_hbm, wgbuf, GS), u=(wu_hbm, wubuf, US))[kind]
            return rows_desc(src, dst, a, s)

        pb = [plist[i:i + BATCH] for i in range(0, len(plist), BATCH)]
        cnt = [0]
        def pissue(i):
            if i < len(pb):
                for d in pb[i]:
                    pdesc(d).start(priority=cnt[0] % 2)
                    cnt[0] += 1
                    if cnt[0] == 1:
                        pltpu.make_async_copy(x_hbm, xbuf, sem.at[XS]).start(priority=1)
                        pltpu.make_async_copy(gw_hbm, gwbuf, sem.at[XS]).start(priority=0)
            else:
                issue(False, 0, i - len(pb))

        waited = {}
        def pwait(i):
            kinds = {}
            for kind, _ in pb[i]:
                kinds[kind] = kinds.get(kind, 0) + 1
            for kind, n in kinds.items():
                s = dict(q=QS, g=GS, u=US)[kind]
                done = waited.get(kind, 0)
                waited[kind] = done + n
                if kind == "q":
                    assert n % 2 == 0 and done % 2 == 0
                    wait_on(wqbuf.at[pl.ds(done * 4, n * 4), :], s)
                else:
                    ref = dict(g=wgbuf, u=wubuf)[kind]
                    wait_on(ref.at[pl.ds(done * WR, n * WR), :], s)

        total = {}
        for kind, _ in plist:
            total[kind] = total.get(kind, 0) + 1
        for i in range(dp):
            pissue(i)
        done_c = set()
        row = lax.broadcasted_iota(jnp.int32, (GH, GW), 0)
        col = lax.broadcasted_iota(jnp.int32, (GH, GW), 1)
        diag = (col // DH) == row
        gate = None
        sg = None
        for i in range(len(pb)):
            pwait(i)
            pissue(i + dp)
            if i == 0:
                wait_on(xbuf, XS)
                wait_on(gwbuf, XS)
                xf = xbuf[0].astype(jnp.float32)
                gw = gwbuf[...].astype(jnp.float32).reshape(1, D)
                gate = jax.nn.sigmoid(jnp.sum(xf * gw, axis=-1, keepdims=True))
            if not compute:
                continue
            x8 = jnp.broadcast_to(xbuf[0], (8, D))
            if "q" not in done_c and waited.get("q", 0) == total["q"]:
                done_c.add("q")
                for g in range(NG):
                    q8 = jnp.dot(x8, wqbuf[:, g * GW:(g + 1) * GW], preferred_element_type=jnp.float32)
                    qscr[g] = jnp.where(diag, q8, 0.0).astype(jnp.bfloat16)
            if "g" not in done_c and waited.get("g", 0) == total["g"]:
                done_c.add("g")
                gg = lax.dot_general(x8, wgbuf[...], NT, preferred_element_type=jnp.float32)
                sg = gg * jax.nn.sigmoid(gg)
            if "u" not in done_c and waited.get("u", 0) == total["u"] and "g" in done_c:
                done_c.add("u")
                uu = lax.dot_general(x8, wubuf[...], NT, preferred_element_type=jnp.float32)
                hscr[...] = (sg * uu).astype(jnp.bfloat16)

        def group(g, carry):
            def kstep(c, carry):
                slot = c % NB
                wait_on(ring.at[slot], slot)
                @pl.when(c + dp < PER)
                def _():
                    issue(False, g, c + dp)
                @pl.when(c + dp >= PER)
                def _():
                    issue(True, g, c + dp - PER)
                if compute:
                    s = None
                    for j in range(GH):
                        t = lax.dot_general(qscr[g, :, j * DH:(j + 1) * DH], ring[slot, j], NT,
                                            preferred_element_type=jnp.float32)
                        s = t if s is None else s + t
                    sscr[c] = s
                return carry
            lax.fori_loop(0, PER, kstep, 0)

            if compute:
                s = sscr[...] * scale
                m = jnp.max(jnp.max(s, axis=0), axis=-1, keepdims=True)
                p = jnp.exp(s - m[None])
                l = jnp.sum(jnp.sum(p, axis=0), axis=-1, keepdims=True)
                pscr[...] = p.astype(jnp.bfloat16)

            def vstep(c, o):
                slot = c % NB
                wait_on(ring.at[slot], slot)
                @pl.when(c + dp < PER)
                def _():
                    issue(True, g, c + dp)
                @pl.when(jnp.logical_and(c + dp >= PER, g < NG - 1))
                def _():
                    issue(False, g + 1, c + dp - PER)
                for e in range(min(dp, NE)):
                    @pl.when(jnp.logical_and(c + dp == PER + e, g == NG - 1))
                    def _():
                        eissue(e)
                if not compute:
                    return o
                pc = pscr[c]
                parts = [jnp.dot(pc, ring[slot, j], preferred_element_type=jnp.float32) for j in range(GH)]
                return o + jnp.concatenate(parts, axis=1)
            o = lax.fori_loop(0, PER, vstep, jnp.zeros((GH, GW), jnp.float32))
            if compute:
                oscr[g] = jnp.where(diag, o / l, 0.0).astype(jnp.bfloat16)
            return carry

        lax.fori_loop(0, NG, group, 0)

        a = jnp.zeros((GH, D), jnp.float32)
        for e in range(NWO):
            wait_on(wobuf.at[e], OS + e)
            if e + dp < NE:
                eissue(e + dp)
            if compute:
                for j in range(8):
                    h = 4 * j + e
                    a = a + jnp.dot(oscr[h // GH, :, (h % GH) * DH:(h % GH + 1) * DH], wobuf[e, j],
                                    preferred_element_type=jnp.float32)
        acc = gate * jnp.sum(a, axis=0, keepdims=True)
        omg = 1.0 - gate
        for i in range(npiece):
            lo, hi = splits[i], splits[i + 1]
            wait_on(wdbuf.at[pl.ds(lo, hi - lo), :], DS + i)
            if compute:
                acc = acc + omg * jnp.dot(hscr[:, lo:hi], wdbuf[lo:hi, :], preferred_element_type=jnp.float32)[0:1]
        out_ref[0] = acc.astype(out_ref.dtype)
    return kernel


def build(dsc=True, dbc=True, **kw):
    nsub = kw.get("nsub", 4); dp = kw.get("dp", 7)
    npiece = len(kw.get("splits", (0, 896, 1152, 1376))) - 1
    @jax.jit
    def fn(A_x, A_k_cache, A_v_cache, A_wq, A_wo, B_x, B_w_gate, B_w_up, B_w_down, gate_w):
        SK = A_k_cache.shape[2]
        W = min(4096, max(256, SK // 4))
        bf = jnp.bfloat16
        BK = ROWS * nsub
        PER = W // BK
        anyspec = pl.BlockSpec(memory_space=pl.ANY)
        return pl.pallas_call(
            make_kernel(SK, W, **kw),
            out_shape=jax.ShapeDtypeStruct((1, 1, D), bf),
            in_specs=[anyspec] * 9,
            out_specs=pl.BlockSpec(memory_space=pltpu.VMEM),
            scratch_shapes=[
                pltpu.VMEM((1, 1, D), bf), pltpu.VMEM((D,), bf),
                pltpu.VMEM((dp + 1, GH, BK, DH), bf),
                pltpu.VMEM((D, H * DH), bf), pltpu.VMEM((4, 8, DH, D), bf),
                pltpu.VMEM((F, D), bf), pltpu.VMEM((F, D), bf), pltpu.VMEM((F, D), bf),
                pltpu.VMEM((NG, GH, GW), bf), pltpu.VMEM((PER, GH, BK), jnp.float32), pltpu.VMEM((PER, GH, BK), bf),
                pltpu.VMEM((8, F), bf), pltpu.VMEM((NG, GH, GW), bf),
                pltpu.SemaphoreType.DMA((dp + 1 + 4 + 4 + npiece,)),
            ],
            compiler_params=pltpu.CompilerParams(vmem_limit_bytes=64 * 1024 * 1024,
                                                 disable_semaphore_checks=dsc, disable_bounds_checks=dbc),
        )(A_x, gate_w, A_k_cache, A_v_cache, A_wq, A_wo, B_w_gate.T, B_w_up.T, B_w_down)
    return fn


_impl = build()


@jax.jit
def pallas_gated_mix__sliding_block_cached__swiglu_ffn__decode_kernel(
    A_x: jax.Array,
    A_k_cache: jax.Array,
    A_v_cache: jax.Array,
    A_wq: jax.Array,
    A_wo: jax.Array,
    B_x: jax.Array,
    B_w_gate: jax.Array,
    B_w_up: jax.Array,
    B_w_down: jax.Array,
    gate_w: jax.Array,
):
    return _impl(A_x, A_k_cache, A_v_cache, A_wq, A_wo, B_x, B_w_gate, B_w_up, B_w_down, gate_w)
```

```python
import jax
import jax.numpy as jnp
from jax import lax
import jax.experimental.pallas as pl
import jax.experimental.pallas.tpu as pltpu

H, DH, D, F = 32, 128, 512, 1376
NT = (((1,), (1,)), ((), ()))
ROWS = 128
UT = 16
BATCH = 32


def _rr(streams):
    out = []
    for k in range(max(len(s) for s in streams)):
        for s in streams:
            if k < len(s):
                out.append(s[k])
    return out


def _rects(t0, t1, tb):
    out = []
    while t0 < t1:
        b, c = divmod(t0, tb)
        if c == 0 and t1 - t0 >= tb:
            nb = (t1 - t0) // tb
            out.append((8 * b, 8 * nb, 0, tb * 128))
            t0 += nb * tb
        else:
            e = min(t1, (b + 1) * tb)
            out.append((8 * b, 8, c * 128, (e - t0) * 128))
            t0 = e
    return out


def _units(nrows, ncols, o):
    tb = ncols // 128
    T = nrows // 8 * tb
    assert T % UT == 0
    us = []
    for u in range(T // UT):
        if u == 0:
            us.append((_rects(T - o, T, tb) if o else []) + _rects(0, UT - o, tb))
        else:
            us.append(_rects(u * UT - o, (u + 1) * UT - o, tb))
    return us


def _streams_of(n, stride):
    return [list(range(s, min(s + stride, n))) for s in range(0, n, stride)]


def make_kernel(SK, W, GH=16, dp=3, NB=4, t0units=20, splits=(0, 896, 1152, 1376), compute=True,
                ffn="C", S=16, oq=2, oo=2, of=3, od=3, LA=128, pchunk=16, atsplit=True):
    scale = DH ** -0.5
    NG = H // GH
    GW = GH * DH
    nsub = BATCH // GH
    BK = ROWS * nsub
    PER = W // BK
    assert PER % NB == 0 and 2 <= dp < NB <= PER
    npiece = len(splits) - 1
    NWO = 4

    def kernel(x_hbm, gw_hbm, k_hbm, v_hbm, wq_hbm, wo_hbm, wg_hbm, wu_hbm, wd_hbm, out_ref,
               xbuf, gwbuf, ring, wqbuf, wobuf, wgbuf, wubuf, wdbuf, qscr, sscr, pscr, hscr, oscr,
               sem):
        XS, QS, GS, US = NB, NB + 1, NB + 2, NB + 3
        OS = NB + 4
        DS = OS + NWO

        def wait_on(ref, s):
            pltpu.make_async_copy(ref, ref, sem.at[s]).wait()

        def al(v, m):
            return v if isinstance(v, int) else pl.multiple_of(v, m)

        def issue(is_v, g, c):
            src = v_hbm if is_v else k_hbm
            slot = c % NB
            n = 0
            for sub in range(nsub):
                for j in range(GH):
                    h = g * GH + j
                    def cp(src_row, dst_row, nrows, n=n, h=h, j=j):
                        pltpu.make_async_copy(src.at[0, h, pl.ds(src_row, nrows), :],
                                              ring.at[slot, j, pl.ds(dst_row, nrows), :],
                                              sem.at[slot]).start(priority=n % 2)
                    if sub == 0 and S:
                        if atsplit:
                            cp(al(SK - W + (c * BK + W - S) % W, 8), 0, S)
                            cp(al(SK - W + c * BK, 8), S, ROWS - S)
                        elif isinstance(c, int):
                            if c == 0:
                                cp(SK - S, 0, S); cp(SK - W, S, ROWS - S)
                            else:
                                cp(SK - W - S + c * BK, 0, ROWS)
                        else:
                            @pl.when(c == 0)
                            def _():
                                cp(SK - S, 0, S); cp(SK - W, S, ROWS - S)
                            @pl.when(c != 0)
                            def _():
                                cp(al(SK - W - S + c * BK, 8), 0, ROWS)
                    else:
                        cp(al(SK - W - S + c * BK + sub * ROWS, 8), sub * ROWS, ROWS)
                    n += 1
        kv_descs = BATCH + (GH if (S and atsplit) else 0)

        def mk(src, dst, s, pr):
            return lambda: pltpu.make_async_copy(src, dst, sem.at[s]).start(priority=pr)

        def rect_desc(src, dst, rect, s, pr):
            r, nr, c, nc = rect
            return mk(src.at[pl.ds(r, nr), pl.ds(c, nc)], dst.at[pl.ds(r, nr), pl.ds(c, nc)], s, pr)

        wo_units = _units(H * DH, D, oo)
        wd_units = _units(F, D, od)
        eunits = []
        for n, u in enumerate(_rr(_streams_of(len(wo_units), 16))):
            th = []
            for (r, nr, c, nc) in wo_units[u]:
                j, rem = divmod(r, 512)
                eb, lr = divmod(rem, DH)
                th.append(mk(wo_hbm.at[pl.ds(r, nr), pl.ds(c, nc)], wobuf.at[eb, j, pl.ds(lr, nr), pl.ds(c, nc)], OS + eb, n % 2))
            eunits.append(th)
        def piece(r):
            return max(i for i in range(npiece) if splits[i] <= r)
        t0 = list(range(0, t0units)); t1 = list(range(t0units, len(wd_units)))
        for k in range(max(len(t0), len(t1))):
            for lst, pr in ((t0, 0), (t1, 1)):
                if k < len(lst):
                    eunits.append([rect_desc(wd_hbm, wdbuf, rect, DS + piece(rect[0]), pr) for rect in wd_units[lst[k]]])
        ecum = [0]
        for th in eunits:
            ecum.append(ecum[-1] + len(th))
        eptr = [0]
        def e_take(upto_desc):
            out = []
            while eptr[0] < len(eunits) and ecum[eptr[0] + 1] <= upto_desc:
                out.append(eunits[eptr[0]]); eptr[0] += 1
            return out
        def run(units):
            for th in units:
                for t in th:
                    t()

        wq_units = _units(D, H * DH, oq)
        f_units = _units(F, D, of)
        nf = len(f_units)
        plist = [("q", u) for u in _rr(_streams_of(len(wq_units), 16))]
        if ffn == "B":
            plist += _rr([[("g", u) for u in s] for s in _streams_of(nf, 16)] + [[("u", u) for u in s] for s in _streams_of(nf, 16)])
        elif ffn == "C":
            plist += _rr([[("g", u) for u in s] for s in _streams_of(nf, 8)] + [[("u", u) for u in s] for s in _streams_of(nf, 8)])
        pinfo = dict(q=(wq_hbm, wqbuf, QS, wq_units, 4), g=(wg_hbm, wgbuf, GS, f_units, 32), u=(wu_hbm, wubuf, US, f_units, 32))
        pitems = []
        for n, (kind, u) in enumerate(plist):
            src, dst, s, units, _ = pinfo[kind]
            th = [rect_desc(src, dst, rect, s, n % 2) for rect in units[u]]
            if n == 0:
                th += [mk(x_hbm, xbuf, XS, 0), mk(gw_hbm, gwbuf, XS, 0)]
            pitems.append((len(th), th))
        for c in range(dp):
            pitems.append((kv_descs, [lambda c=c: issue(False, 0, c)]))
        pcum = [0]
        for nd, _ in pitems:
            pcum.append(pcum[-1] + nd)
        pptr = [0]
        def p_issue(upto_desc):
            while pptr[0] < len(pitems) and pcum[pptr[0] + 1] <= upto_desc:
                for t in pitems[pptr[0]][1]:
                    t()
                pptr[0] += 1

        total = {}
        for kind, _ in plist:
            total[kind] = total.get(kind, 0) + 1
        waited = {}
        done_c = set()
        row = lax.broadcasted_iota(jnp.int32, (GH, GW), 0)
        col = lax.broadcasted_iota(jnp.int32, (GH, GW), 1)
        diag = (col // DH) == row
        row1 = lax.broadcasted_iota(jnp.int32, (GH, DH), 0)
        gate = None
        sg = None
        p_issue(LA)
        i = 0
        while i < len(plist):
            e = i
            while e < len(plist) and (pcum[e + 1] - pcum[i] <= 3 * pchunk or (e - i) % 2 == 1):
                e += 1
            assert pptr[0] >= e, "chunk must be issued before waiting"
            kinds = {}
            for kind, _ in plist[i:e]:
                kinds[kind] = kinds.get(kind, 0) + 1
            for kind, n in kinds.items():
                _, dst, s, _, rpu = pinfo[kind]
                done = waited.get(kind, 0)
                waited[kind] = done + n
                assert (done * rpu) % 8 == 0 and (n * rpu) % 8 == 0, (kind, done, n)
                wait_on(dst.at[pl.ds(done * rpu, n * rpu), :], s)
            p_issue(pcum[e] + LA if e < len(plist) else 10 ** 9)
            if i == 0:
                wait_on(xbuf, XS)
                wait_on(gwbuf, XS)
                xf = xbuf[0].astype(jnp.float32)
                gw = gwbuf[...].astype(jnp.float32).reshape(1, D)
                gate = jax.nn.sigmoid(jnp.sum(xf * gw, axis=-1, keepdims=True))
            i = e
            if not compute:
                continue
            qdone = waited.get("q", 0) == total["q"]
            nq = [g for g in range(H // 8) if ("q", g) not in done_c]
            if qdone and nq:
                for g8 in (nq if i >= len(plist) else nq[:1]):
                    done_c.add(("q", g8))
                    g, part = divmod(g8 * 8, GH)
                    lo = part * DH
                    xg = jnp.broadcast_to(xbuf[0], (GH, D))
                    qg = jnp.dot(xg, wqbuf[:, g8 * 1024:(g8 + 1) * 1024], preferred_element_type=jnp.float32)
                    qscr[g, :, lo:lo + 1024] = jnp.where(diag[:, lo:lo + 1024], qg, 0.0).astype(jnp.bfloat16)
            x8 = jnp.broadcast_to(xbuf[0], (8, D))
            if "g" not in done_c and waited.get("g", 0) == total["g"]:
                done_c.add("g")
                gg = lax.dot_general(x8, wgbuf[...], NT, preferred_element_type=jnp.float32)
                sg = gg * jax.nn.sigmoid(gg)
            if "u" not in done_c and waited.get("u", 0) == total["u"] and "g" in done_c:
                done_c.add("u")
                uu = lax.dot_general(x8, wubuf[...], NT, preferred_element_type=jnp.float32)
                hscr[...] = (sg * uu).astype(jnp.bfloat16)
        assert pptr[0] == len(pitems)

        inloop = []
        for e in range(dp):
            inloop.append(e_take(max(LA - (dp - 1 - e) * kv_descs, 0)))

        def group(g, carry):
            def kstep(c, carry):
                slot = c % NB
                wait_on(ring.at[slot], slot)
                @pl.when(c + dp < PER)
                def _():
                    issue(False, g, c + dp)
                @pl.when(c + dp >= PER)
                def _():
                    issue(True, g, c + dp - PER)
                if compute:
                    s = None
                    for j in range(GH):
                        t = lax.dot_general(qscr[g, :, j * DH:(j + 1) * DH], ring[slot, j], NT,
                                            preferred_element_type=jnp.float32)
                        s = t if s is None else s + t
                    sscr[c] = s
                return carry
            lax.fori_loop(0, PER, kstep, 0)

            if compute:
                s = sscr[...] * scale
                m = jnp.max(jnp.max(s, axis=0), axis=-1, keepdims=True)
                p = jnp.exp(s - m[None])
                l = jnp.sum(jnp.sum(p, axis=0), axis=-1, keepdims=True)
                pscr[...] = p.astype(jnp.bfloat16)

            def vstep(c, o):
                slot = c % NB
                wait_on(ring.at[slot], slot)
                @pl.when(c + dp < PER)
                def _():
                    issue(True, g, c + dp)
                @pl.when(jnp.logical_and(c + dp >= PER, g < NG - 1))
                def _():
                    issue(False, g + 1, c + dp - PER)
                for e in range(dp):
                    if inloop[e]:
                        @pl.when(jnp.logical_and(c + dp == PER + e, g == NG - 1))
                        def _():
                            run(inloop[e])
                if not compute:
                    return o
                pc = pscr[c]
                for j in range(GH):
                    t = jnp.dot(pc, ring[slot, j], preferred_element_type=jnp.float32)
                    o = o + jnp.where(row1 == j, t, 0.0)
                return o
            o = lax.fori_loop(0, PER, vstep, jnp.zeros((GH, DH), jnp.float32))
            if compute:
                oscr[g] = o / l
            return carry

        lax.fori_loop(0, NG, group, 0)

        a = jnp.zeros((GH, D), jnp.float32)
        nparts = BATCH // pchunk
        for e in range(NWO):
            for part in range(nparts):
                need = min((e + 1) * BATCH + 8, len(wo_units)) if part == nparts - 1 else e * BATCH + (part + 1) * pchunk + 8
                if eptr[0] < need:
                    run(e_take(ecum[need]))
                jn = 8 // nparts
                wait_on(wobuf.at[e, pl.ds(part * jn, jn)], OS + e)
                run(e_take(ecum[e * BATCH + (part + 1) * pchunk] + LA))
            if compute:
                for j in range(8):
                    h = 4 * j + e
                    lhs = jnp.where(row1 == h % GH, oscr[h // GH], 0.0).astype(jnp.bfloat16)
                    a = a + jnp.dot(lhs, wobuf[e, j], preferred_element_type=jnp.float32)
        run(e_take(10 ** 9))
        assert eptr[0] == len(eunits)
        acc = gate * jnp.sum(a, axis=0, keepdims=True)
        omg = 1.0 - gate
        for i in range(npiece):
            lo, hi = splits[i], splits[i + 1]
            wait_on(wdbuf.at[pl.ds(lo, hi - lo), :], DS + i)
            if compute:
                acc = acc + omg * jnp.dot(hscr[:, lo:hi], wdbuf[lo:hi, :], preferred_element_type=jnp.float32)[0:1]
        out_ref[0] = acc.astype(out_ref.dtype)
    return kernel


def build(dsc=True, dbc=True, **kw):
    GH = kw.get("GH", 16); NB = kw.get("NB", 4)
    npiece = len(kw.get("splits", (0, 896, 1152, 1376))) - 1
    @jax.jit
    def fn(A_x, A_k_cache, A_v_cache, A_wq, A_wo, B_x, B_w_gate, B_w_up, B_w_down, gate_w):
        SK = A_k_cache.shape[2]
        W = min(4096, max(256, SK // 4))
        bf = jnp.bfloat16
        BK = ROWS * BATCH // GH
        PER = W // BK
        NG = H // GH
        anyspec = pl.BlockSpec(memory_space=pl.ANY)
        return pl.pallas_call(
            make_kernel(SK, W, **kw),
            out_shape=jax.ShapeDtypeStruct((1, 1, D), bf),
            in_specs=[anyspec] * 9,
            out_specs=pl.BlockSpec(memory_space=pltpu.VMEM),
            scratch_shapes=[
                pltpu.VMEM((1, 1, D), bf), pltpu.VMEM((D,), bf),
                pltpu.VMEM((NB, GH, BK, DH), bf),
                pltpu.VMEM((D, H * DH), bf), pltpu.VMEM((4, 8, DH, D), bf),
                pltpu.VMEM((F, D), bf), pltpu.VMEM((F, D), bf), pltpu.VMEM((F, D), bf),
                pltpu.VMEM((NG, GH, GH * DH), bf), pltpu.VMEM((PER, GH, BK), jnp.float32), pltpu.VMEM((PER, GH, BK), bf),
                pltpu.VMEM((8, F), bf), pltpu.VMEM((NG, GH, DH), jnp.float32),
                pltpu.SemaphoreType.DMA((NB + 4 + 4 + npiece,)),
            ],
            compiler_params=pltpu.CompilerParams(vmem_limit_bytes=64 * 1024 * 1024,
                                                 disable_semaphore_checks=dsc, disable_bounds_checks=dbc),
        )(A_x, gate_w, A_k_cache, A_v_cache, A_wq, A_wo, B_w_gate.T, B_w_up.T, B_w_down)
    return fn


_impl = build(LA=192, S=0)


@jax.jit
def pallas_gated_mix__sliding_block_cached__swiglu_ffn__decode_kernel(
    A_x: jax.Array,
    A_k_cache: jax.Array,
    A_v_cache: jax.Array,
    A_wq: jax.Array,
    A_wo: jax.Array,
    B_x: jax.Array,
    B_w_gate: jax.Array,
    B_w_up: jax.Array,
    B_w_down: jax.Array,
    gate_w: jax.Array,
):
    return _impl(A_x, A_k_cache, A_v_cache, A_wq, A_wo, B_x, B_w_gate, B_w_up, B_w_down, gate_w)
```

```python
import jax
import jax.numpy as jnp
from jax import lax
import jax.experimental.pallas as pl
import jax.experimental.pallas.tpu as pltpu

H, DH, D, F = 32, 128, 512, 1376
NT = (((1,), (1,)), ((), ()))
ROWS = 128
UT = 16
BATCH = 32


def _rr(streams):
    out = []
    for k in range(max(len(s) for s in streams)):
        for s in streams:
            if k < len(s):
                out.append(s[k])
    return out


def _rects(t0, t1, tb):
    out = []
    while t0 < t1:
        b, c = divmod(t0, tb)
        if c == 0 and t1 - t0 >= tb:
            nb = (t1 - t0) // tb
            out.append((8 * b, 8 * nb, 0, tb * 128))
            t0 += nb * tb
        else:
            e = min(t1, (b + 1) * tb)
            out.append((8 * b, 8, c * 128, (e - t0) * 128))
            t0 = e
    return out


def _units(nrows, ncols, o):
    tb = ncols // 128
    T = nrows // 8 * tb
    assert T % UT == 0
    us = []
    for u in range(T // UT):
        if u == 0:
            us.append((_rects(T - o, T, tb) if o else []) + _rects(0, UT - o, tb))
        else:
            us.append(_rects(u * UT - o, (u + 1) * UT - o, tb))
    return us


def _streams_of(n, stride):
    return [list(range(s, min(s + stride, n))) for s in range(0, n, stride)]


def make_kernel(SK, W, GH=16, dp=3, NB=4, t0units=20, splits=(0, 896, 1152, 1272, 1336, 1376), compute=True,
                ffn="C", S=16, oq=2, oo=2, of=3, od=3, LA=192, pchunk=16, atsplit=True, vlo=1152):
    scale = DH ** -0.5
    NG = H // GH
    GW = GH * DH
    nsub = BATCH // GH
    BK = ROWS * nsub
    PER = W // BK
    assert PER % NB == 0 and 2 <= dp < NB <= PER
    npiece = len(splits) - 1
    NWO = 4

    def kernel(x_hbm, gw_hbm, k_hbm, v_hbm, wq_hbm, wo_hbm, wg_hbm, wu_hbm, wd_hbm, out_ref,
               xbuf, gwbuf, ring, wqbuf, wobuf, wgbuf, wubuf, wdbuf, qscr, sscr, pscr, hscr, oscr, hcscr,
               sem):
        XS, QS, GS, US = NB, NB + 1, NB + 2, NB + 3
        OS = NB + 4
        DS = OS + NWO

        def wait_on(ref, s):
            pltpu.make_async_copy(ref, ref, sem.at[s]).wait()

        def al(v, m):
            return v if isinstance(v, int) else pl.multiple_of(v, m)

        def issue(is_v, g, c):
            src = v_hbm if is_v else k_hbm
            slot = c % NB
            n = 0
            for sub in range(nsub):
                for j in range(GH):
                    h = g * GH + j
                    def cp(src_row, dst_row, nrows, n=n, h=h, j=j):
                        pltpu.make_async_copy(src.at[0, h, pl.ds(src_row, nrows), :],
                                              ring.at[slot, j, pl.ds(dst_row, nrows), :],
                                              sem.at[slot]).start(priority=n % 2)
                    if sub == 0 and S:
                        if atsplit:
                            cp(al(SK - W + (c * BK + W - S) % W, 8), 0, S)
                            cp(al(SK - W + c * BK, 8), S, ROWS - S)
                        elif isinstance(c, int):
                            if c == 0:
                                cp(SK - S, 0, S); cp(SK - W, S, ROWS - S)
                            else:
                                cp(SK - W - S + c * BK, 0, ROWS)
                        else:
                            @pl.when(c == 0)
                            def _():
                                cp(SK - S, 0, S); cp(SK - W, S, ROWS - S)
                            @pl.when(c != 0)
                            def _():
                                cp(al(SK - W - S + c * BK, 8), 0, ROWS)
                    else:
                        cp(al(SK - W - S + c * BK + sub * ROWS, 8), sub * ROWS, ROWS)
                    n += 1
        kv_descs = BATCH + (GH if (S and atsplit) else 0)

        def mk(src, dst, s, pr):
            return lambda: pltpu.make_async_copy(src, dst, sem.at[s]).start(priority=pr)

        def rect_desc(src, dst, rect, s, pr):
            r, nr, c, nc = rect
            return mk(src.at[pl.ds(r, nr), pl.ds(c, nc)], dst.at[pl.ds(r, nr), pl.ds(c, nc)], s, pr)

        wo_units = _units(H * DH, D, oo)
        wd_units = _units(F, D, od)
        eunits = []
        for n, u in enumerate(_rr(_streams_of(len(wo_units), 16))):
            th = []
            for (r, nr, c, nc) in wo_units[u]:
                j, rem = divmod(r, 512)
                eb, lr = divmod(rem, DH)
                th.append(mk(wo_hbm.at[pl.ds(r, nr), pl.ds(c, nc)], wobuf.at[eb, j, pl.ds(lr, nr), pl.ds(c, nc)], OS + eb, n % 2))
            eunits.append(th)
        def piece(r):
            return max(i for i in range(npiece) if splits[i] <= r)
        t0 = list(range(0, t0units)); t1 = list(range(t0units, len(wd_units)))
        for k in range(max(len(t0), len(t1))):
            for lst, pr in ((t0, 0), (t1, 1)):
                if k < len(lst):
                    eunits.append([rect_desc(wd_hbm, wdbuf, rect, DS + piece(rect[0]), pr) for rect in wd_units[lst[k]]])
        ecum = [0]
        for th in eunits:
            ecum.append(ecum[-1] + len(th))
        eptr = [0]
        def e_take(upto_desc):
            out = []
            while eptr[0] < len(eunits) and ecum[eptr[0] + 1] <= upto_desc:
                out.append(eunits[eptr[0]]); eptr[0] += 1
            return out
        def run(units):
            for th in units:
                for t in th:
                    t()

        wq_units = _units(D, H * DH, oq)
        f_units = _units(F, D, of)
        nf = len(f_units)
        plist = [("q", u) for u in _rr(_streams_of(len(wq_units), 16))]
        if ffn == "B":
            plist += _rr([[("g", u) for u in s] for s in _streams_of(nf, 16)] + [[("u", u) for u in s] for s in _streams_of(nf, 16)])
        elif ffn == "C":
            plist += _rr([[("g", u) for u in s] for s in _streams_of(nf, 8)] + [[("u", u) for u in s] for s in _streams_of(nf, 8)])
        pinfo = dict(q=(wq_hbm, wqbuf, QS, wq_units, 4), g=(wg_hbm, wgbuf, GS, f_units, 32), u=(wu_hbm, wubuf, US, f_units, 32))
        pitems = []
        for n, (kind, u) in enumerate(plist):
            src, dst, s, units, _ = pinfo[kind]
            th = [rect_desc(src, dst, rect, s, n % 2) for rect in units[u]]
            if n == 0:
                th += [mk(x_hbm, xbuf, XS, 0), mk(gw_hbm, gwbuf, XS, 0)]
            pitems.append((len(th), th))
        for c in range(dp):
            pitems.append((kv_descs, [lambda c=c: issue(False, 0, c)]))
        pcum = [0]
        for nd, _ in pitems:
            pcum.append(pcum[-1] + nd)
        pptr = [0]
        def p_issue(upto_desc):
            while pptr[0] < len(pitems) and pcum[pptr[0] + 1] <= upto_desc:
                for t in pitems[pptr[0]][1]:
                    t()
                pptr[0] += 1

        total = {}
        for kind, _ in plist:
            total[kind] = total.get(kind, 0) + 1
        waited = {}
        done_c = set()
        row = lax.broadcasted_iota(jnp.int32, (GH, GW), 0)
        col = lax.broadcasted_iota(jnp.int32, (GH, GW), 1)
        diag = (col // DH) == row
        row1 = lax.broadcasted_iota(jnp.int32, (GH, DH), 0)
        gate = None
        sg = None
        p_issue(LA)
        i = 0
        while i < len(plist):
            e = i
            while e < len(plist) and (pcum[e + 1] - pcum[i] <= 3 * pchunk or (e - i) % 2 == 1):
                e += 1
            assert pptr[0] >= e, "chunk must be issued before waiting"
            kinds = {}
            for kind, _ in plist[i:e]:
                kinds[kind] = kinds.get(kind, 0) + 1
            for kind, n in kinds.items():
                _, dst, s, _, rpu = pinfo[kind]
                done = waited.get(kind, 0)
                waited[kind] = done + n
                assert (done * rpu) % 8 == 0 and (n * rpu) % 8 == 0, (kind, done, n)
                wait_on(dst.at[pl.ds(done * rpu, n * rpu), :], s)
            p_issue(pcum[e] + LA if e < len(plist) else 10 ** 9)
            if i == 0:
                wait_on(xbuf, XS)
                wait_on(gwbuf, XS)
                xf = xbuf[0].astype(jnp.float32)
                gw = gwbuf[...].astype(jnp.float32).reshape(1, D)
                gate = jax.nn.sigmoid(jnp.sum(xf * gw, axis=-1, keepdims=True))
            i = e
            if not compute:
                continue
            qdone = waited.get("q", 0) == total["q"]
            nq = [g for g in range(H // 8) if ("q", g) not in done_c]
            if qdone and nq:
                for g8 in (nq if i >= len(plist) else nq[:1]):
                    done_c.add(("q", g8))
                    g, part = divmod(g8 * 8, GH)
                    lo = part * DH
                    xg = jnp.broadcast_to(xbuf[0], (GH, D))
                    qg = jnp.dot(xg, wqbuf[:, g8 * 1024:(g8 + 1) * 1024], preferred_element_type=jnp.float32)
                    qscr[g, :, lo:lo + 1024] = jnp.where(diag[:, lo:lo + 1024], qg, 0.0).astype(jnp.bfloat16)
            x8 = jnp.broadcast_to(xbuf[0], (8, D))
            if "g" not in done_c and waited.get("g", 0) == total["g"]:
                done_c.add("g")
                gg = lax.dot_general(x8, wgbuf[...], NT, preferred_element_type=jnp.float32)
                sg = gg * jax.nn.sigmoid(gg)
            if "u" not in done_c and waited.get("u", 0) == total["u"] and "g" in done_c:
                done_c.add("u")
                uu = lax.dot_general(x8, wubuf[...], NT, preferred_element_type=jnp.float32)
                hh = (sg * uu).astype(jnp.bfloat16)
                hscr[...] = hh
                if vlo < F:
                    nv = F - vlo
                    eye = lax.broadcasted_iota(jnp.int32, (nv, nv), 0) == lax.broadcasted_iota(jnp.int32, (nv, nv), 1)
                    hrow = jnp.broadcast_to(hh[0:1, vlo:F].astype(jnp.float32), (nv, nv))
                    dm = jnp.where(eye, hrow, 0.0).astype(jnp.bfloat16)
                    hcscr[...] = jnp.dot(dm, jnp.ones((nv, DH), jnp.bfloat16), preferred_element_type=jnp.float32) * (1.0 - gate)
        assert pptr[0] == len(pitems)

        inloop = []
        for e in range(dp):
            inloop.append(e_take(max(LA - (dp - 1 - e) * kv_descs, 0)))

        def group(g, carry):
            def kstep(c, carry):
                slot = c % NB
                wait_on(ring.at[slot], slot)
                @pl.when(c + dp < PER)
                def _():
                    issue(False, g, c + dp)
                @pl.when(c + dp >= PER)
                def _():
                    issue(True, g, c + dp - PER)
                if compute:
                    s = None
                    for j in range(GH):
                        t = lax.dot_general(qscr[g, :, j * DH:(j + 1) * DH], ring[slot, j], NT,
                                            preferred_element_type=jnp.float32)
                        s = t if s is None else s + t
                    sscr[c] = s
                return carry
            lax.fori_loop(0, PER, kstep, 0)

            if compute:
                s = sscr[...] * scale
                m = jnp.max(jnp.max(s, axis=0), axis=-1, keepdims=True)
                p = jnp.exp(s - m[None])
                l = jnp.sum(jnp.sum(p, axis=0), axis=-1, keepdims=True)
                pscr[...] = p.astype(jnp.bfloat16)

            def vstep(c, o):
                slot = c % NB
                wait_on(ring.at[slot], slot)
                @pl.when(c + dp < PER)
                def _():
                    issue(True, g, c + dp)
                @pl.when(jnp.logical_and(c + dp >= PER, g < NG - 1))
                def _():
                    issue(False, g + 1, c + dp - PER)
                for e in range(dp):
                    if inloop[e]:
                        @pl.when(jnp.logical_and(c + dp == PER + e, g == NG - 1))
                        def _():
                            run(inloop[e])
                if not compute:
                    return o
                pc = pscr[c]
                for j in range(GH):
                    t = jnp.dot(pc, ring[slot, j], preferred_element_type=jnp.float32)
                    o = o + jnp.where(row1 == j, t, 0.0)
                return o
            o = lax.fori_loop(0, PER, vstep, jnp.zeros((GH, DH), jnp.float32))
            if compute:
                oscr[g] = o / l
            return carry

        lax.fori_loop(0, NG, group, 0)

        a = jnp.zeros((GH, D), jnp.float32)
        nparts = BATCH // pchunk
        for e in range(NWO):
            for part in range(nparts):
                need = min((e + 1) * BATCH + 8, len(wo_units)) if part == nparts - 1 else e * BATCH + (part + 1) * pchunk + 8
                if eptr[0] < need:
                    run(e_take(ecum[need]))
                jn = 8 // nparts
                wait_on(wobuf.at[e, pl.ds(part * jn, jn)], OS + e)
                run(e_take(ecum[e * BATCH + (part + 1) * pchunk] + LA))
            if compute:
                for j in range(8):
                    h = 4 * j + e
                    lhs = jnp.where(row1 == h % GH, oscr[h // GH], 0.0).astype(jnp.bfloat16)
                    a = a + jnp.dot(lhs, wobuf[e, j], preferred_element_type=jnp.float32)
        run(e_take(10 ** 9))
        assert eptr[0] == len(eunits)
        acc8 = a[0:8]
        for r in range(8, GH, 8):
            acc8 = acc8 + a[r:r + 8]
        acc8 = gate * acc8
        omg = 1.0 - gate
        row8 = lax.broadcasted_iota(jnp.int32, (8, D), 0)
        for i in range(npiece):
            lo, hi = splits[i], splits[i + 1]
            wait_on(wdbuf.at[pl.ds(lo, hi - lo), :], DS + i)
            if not compute:
                continue
            if lo < vlo:
                assert hi <= vlo
                b = jnp.dot(hscr[:, lo:hi], wdbuf[lo:hi, :], preferred_element_type=jnp.float32)
                acc8 = acc8 + jnp.where(row8 == 0, omg * b, 0.0)
            else:
                w = wdbuf[lo:hi, :].astype(jnp.float32)
                hc = hcscr[lo - vlo:hi - vlo, :]
                prod = w * jnp.concatenate([hc] * (D // DH), axis=1)
                acc8 = acc8 + jnp.sum(prod.reshape((hi - lo) // 8, 8, D), axis=0)
        out_ref[0] = jnp.sum(acc8, axis=0, keepdims=True).astype(out_ref.dtype)
    return kernel


def build(dsc=True, dbc=True, **kw):
    GH = kw.get("GH", 16); NB = kw.get("NB", 4)
    npiece = len(kw.get("splits", (0, 896, 1152, 1272, 1336, 1376))) - 1
    vlo = kw.get("vlo", 1152)
    @jax.jit
    def fn(A_x, A_k_cache, A_v_cache, A_wq, A_wo, B_x, B_w_gate, B_w_up, B_w_down, gate_w):
        SK = A_k_cache.shape[2]
        W = min(4096, max(256, SK // 4))
        bf = jnp.bfloat16
        BK = ROWS * BATCH // GH
        PER = W // BK
        NG = H // GH
        anyspec = pl.BlockSpec(memory_space=pl.ANY)
        return pl.pallas_call(
            make_kernel(SK, W, **kw),
            out_shape=jax.ShapeDtypeStruct((1, 1, D), bf),
            in_specs=[anyspec] * 9,
            out_specs=pl.BlockSpec(memory_space=pltpu.VMEM),
            scratch_shapes=[
                pltpu.VMEM((1, 1, D), bf), pltpu.VMEM((D,), bf),
                pltpu.VMEM((NB, GH, BK, DH), bf),
                pltpu.VMEM((D, H * DH), bf), pltpu.VMEM((4, 8, DH, D), bf),
                pltpu.VMEM((F, D), bf), pltpu.VMEM((F, D), bf), pltpu.VMEM((F, D), bf),
                pltpu.VMEM((NG, GH, GH * DH), bf), pltpu.VMEM((PER, GH, BK), jnp.float32), pltpu.VMEM((PER, GH, BK), bf),
                pltpu.VMEM((8, F), bf), pltpu.VMEM((NG, GH, DH), jnp.float32), pltpu.VMEM((max(F - vlo, 8), DH), jnp.float32),
                pltpu.SemaphoreType.DMA((NB + 4 + 4 + npiece,)),
            ],
            compiler_params=pltpu.CompilerParams(vmem_limit_bytes=64 * 1024 * 1024,
                                                 disable_semaphore_checks=dsc, disable_bounds_checks=dbc),
        )(A_x, gate_w, A_k_cache, A_v_cache, A_wq, A_wo, B_w_gate.T, B_w_up.T, B_w_down)
    return fn


_impl = build()


@jax.jit
def pallas_gated_mix__sliding_block_cached__swiglu_ffn__decode_kernel(
    A_x: jax.Array,
    A_k_cache: jax.Array,
    A_v_cache: jax.Array,
    A_wq: jax.Array,
    A_wo: jax.Array,
    B_x: jax.Array,
    B_w_gate: jax.Array,
    B_w_up: jax.Array,
    B_w_down: jax.Array,
    gate_w: jax.Array,
):
    return _impl(A_x, A_k_cache, A_v_cache, A_wq, A_wo, B_x, B_w_gate, B_w_up, B_w_down, gate_w)
```

```python
import jax
import jax.numpy as jnp
from jax import lax
import jax.experimental.pallas as pl
import jax.experimental.pallas.tpu as pltpu

H, DH, D, F = 32, 128, 512, 1376
NT = (((1,), (1,)), ((), ()))

ROWS = 128
UT = 16
BATCH = 32
GH = 16
NG = H // GH
GW = GH * DH
NSUB = BATCH // GH
BK = ROWS * NSUB
DP = 3
NB = 4
LA = 192
PCHUNK = 48
NWO = 4

KV_SHIFT = 16
OFF_A = 2
OFF_B = 3

WD_T0 = 20
WD_SPLITS = (0, 896, 1152, 1272, 1336, 1376)
WD_VPU = 1152
NPIECE = len(WD_SPLITS) - 1


def _round_robin(streams):
    out = []
    for k in range(max(len(s) for s in streams)):
        out += [s[k] for s in streams if k < len(s)]
    return out


def _chop(items, n):
    return [items[i:i + n] for i in range(0, len(items), n)]


def _rects(t0, t1, tb):
    out = []
    while t0 < t1:
        b, c = divmod(t0, tb)
        if c == 0 and t1 - t0 >= tb:
            nb = (t1 - t0) // tb
            out.append((8 * b, 8 * nb, 0, tb * 128))
            t0 += nb * tb
        else:
            e = min(t1, (b + 1) * tb)
            out.append((8 * b, 8, c * 128, (e - t0) * 128))
            t0 = e
    return out


def _units(nrows, ncols, off):
    tb = ncols // 128
    total = nrows // 8 * tb
    assert total % UT == 0
    units = [_rects(total - off, total, tb) + _rects(0, UT - off, tb)]
    units += [_rects(u * UT - off, (u + 1) * UT - off, tb) for u in range(1, total // UT)]
    return units


def _split_cols(rect, parts_per_unit):
    r, nr, c, nc = rect
    nt = nc // 128
    k = max(1, round(nt * parts_per_unit / UT))
    b = [round(nt * i / k) for i in range(k + 1)]
    return [(r, nr, c + 128 * b[i], 128 * (b[i + 1] - b[i])) for i in range(k)]


class _Queue:
    def __init__(self):
        self.items, self.cum, self.ptr = [], [0], 0

    def add(self, starts, ndesc=None):
        self.items.append(starts)
        self.cum.append(self.cum[-1] + (len(starts) if ndesc is None else ndesc))

    def take(self, upto):
        out = []
        while self.ptr < len(self.items) and self.cum[self.ptr + 1] <= upto:
            out += self.items[self.ptr]
            self.ptr += 1
        return out

    def issue(self, upto):
        for start in self.take(upto):
            start()

    def done(self):
        return self.ptr == len(self.items)


def _make_kernel(SK, W):
    scale = DH ** -0.5
    PER = W // BK
    S = KV_SHIFT
    ALL = 1 << 30
    f32, bf16 = jnp.float32, jnp.bfloat16
    assert W % BK == 0 and PER % NB == 0 and 2 <= DP < NB <= PER

    def kernel(x_hbm, gw_hbm, k_hbm, v_hbm, wq_hbm, wo_hbm, wg_hbm, wu_hbm, wd_hbm, out_ref,
               xbuf, gwbuf, ring, wqbuf, wobuf, wgbuf, wubuf, wdbuf,
               qscr, sscr, pscr, hscr, oscr, hcscr, sem):
        XS, QS, GS, US = NB, NB + 1, NB + 2, NB + 3
        OS = NB + 4
        DS = OS + NWO

        def wait_for(ref, s):
            pltpu.make_async_copy(ref, ref, sem.at[s]).wait()

        def start_fn(src, dst, s, prio):
            return lambda: pltpu.make_async_copy(src, dst, sem.at[s]).start(priority=prio)

        def rect_start(src, dst, rect, s, prio):
            r, nr, c, nc = rect
            return start_fn(src.at[pl.ds(r, nr), pl.ds(c, nc)], dst.at[pl.ds(r, nr), pl.ds(c, nc)], s, prio)

        def al8(v):
            return v if isinstance(v, int) else pl.multiple_of(v, 8)

        def issue_kv(src, g, c):
            slot = c % NB
            for sub in range(NSUB):
                for j in range(GH):
                    if sub == 0:
                        parts = [((c * BK + W - S) % W, 0, S), (c * BK, S, ROWS - S)]
                    else:
                        parts = [(c * BK + sub * ROWS - S, sub * ROWS, ROWS)]
                    for src_row, dst_row, n in parts:
                        pltpu.make_async_copy(
                            src.at[0, g * GH + j, pl.ds(al8(SK - W + src_row), n), :],
                            ring.at[slot, j, pl.ds(dst_row, n), :],
                            sem.at[slot]).start(priority=j % 2)

        kv_descs = GH * (NSUB + 1)

        wq_units = _units(D, H * DH, OFF_A)
        wq_order = _round_robin(_chop(list(range(len(wq_units))), 16))
        early = set(wq_order[:16])
        wq_units = [[p for rect in un for p in _split_cols(rect, 8 if u in early else 4)]
                    for u, un in enumerate(wq_units)]
        f_units = _units(F, D, OFF_B)
        nf = len(f_units)
        head_list = [("q", u) for u in wq_order]
        head_list += _round_robin(_chop([("g", u) for u in range(nf)], 8) + _chop([("u", u) for u in range(nf)], 8))
        info = dict(q=(wq_hbm, wqbuf, QS, wq_units, 4), g=(wg_hbm, wgbuf, GS, f_units, 32),
                    u=(wu_hbm, wubuf, US, f_units, 32))
        head = _Queue()
        for n, (kind, u) in enumerate(head_list):
            src, dst, s, units, _ = info[kind]
            starts = [rect_start(src, dst, rect, s, n % 2) for rect in units[u]]
            if n == 0:
                starts += [start_fn(x_hbm, xbuf, XS, 0), start_fn(gw_hbm, gwbuf, XS, 0)]
            head.add(starts)
        for c in range(DP):
            head.add([lambda c=c: issue_kv(k_hbm, 0, c)], kv_descs)

        tail = _Queue()
        wo_units = _units(H * DH, D, OFF_A)
        for n, u in enumerate(_round_robin(_chop(list(range(len(wo_units))), 16))):
            starts = []
            for r, nr, c, nc in wo_units[u]:
                j, rem = divmod(r, NWO * DH)
                e, lr = divmod(rem, DH)
                assert lr + nr <= DH
                starts.append(start_fn(wo_hbm.at[pl.ds(r, nr), pl.ds(c, nc)],
                                       wobuf.at[e, j, pl.ds(lr, nr), pl.ds(c, nc)], OS + e, n % 2))
            tail.add(starts)

        def piece(r):
            return max(i for i in range(NPIECE) if WD_SPLITS[i] <= r)

        assert all(piece(r) == piece(r + nr - 1) for un in f_units for r, nr, _, _ in un)
        for u, prio in _round_robin([[(u, 0) for u in range(WD_T0)], [(u, 1) for u in range(WD_T0, nf)]]):
            tail.add([rect_start(wd_hbm, wdbuf, rect, DS + piece(rect[0]), prio) for rect in f_units[u]])

        row = lax.broadcasted_iota(jnp.int32, (GH, GW), 0)
        col = lax.broadcasted_iota(jnp.int32, (GH, GW), 1)
        diag = (col // DH) == row
        row1 = lax.broadcasted_iota(jnp.int32, (GH, DH), 0)
        total = {k: sum(1 for kind, _ in head_list if kind == k) for k in info}
        waited = {k: 0 for k in info}
        q_todo = list(range(H // 8))
        gate = silu_g = None
        h_done = False
        head.issue(LA)
        i = 0
        while i < len(head_list):
            e = i
            while e < len(head_list) and (head.cum[e + 1] - head.cum[i] <= PCHUNK or (e - i) % 2):
                e += 1
            assert head.ptr >= e
            for kind in info:
                n = sum(1 for k, _ in head_list[i:e] if k == kind)
                if n:
                    _, dst, s, _, rpu = info[kind]
                    assert (waited[kind] * rpu) % 8 == 0 and (n * rpu) % 8 == 0
                    wait_for(dst.at[pl.ds(waited[kind] * rpu, n * rpu), :], s)
                    waited[kind] += n
            head.issue(head.cum[e] + LA if e < len(head_list) else ALL)
            if i == 0:
                wait_for(xbuf, XS)
                wait_for(gwbuf, XS)
                gw = gwbuf[...].astype(f32).reshape(1, D)
                gate = jax.nn.sigmoid(jnp.sum(xbuf[0].astype(f32) * gw, axis=-1, keepdims=True))
            i = e
            if waited["q"] == total["q"]:
                for _ in range(len(q_todo) if i == len(head_list) else min(1, len(q_todo))):
                    g8 = q_todo.pop(0)
                    g, lo = divmod(g8 * 8 * DH, GW)
                    q = jnp.dot(jnp.broadcast_to(xbuf[0], (GH, D)), wqbuf[:, g8 * 8 * DH:(g8 + 1) * 8 * DH],
                                preferred_element_type=f32)
                    qscr[g, :, lo:lo + 8 * DH] = jnp.where(diag[:, lo:lo + 8 * DH], q, 0.0).astype(bf16)
            if silu_g is None and waited["g"] == total["g"]:
                gg = lax.dot_general(jnp.broadcast_to(xbuf[0], (8, D)), wgbuf[...], NT, preferred_element_type=f32)
                silu_g = gg * jax.nn.sigmoid(gg)
            if not h_done and silu_g is not None and waited["u"] == total["u"]:
                h_done = True
                uu = lax.dot_general(jnp.broadcast_to(xbuf[0], (8, D)), wubuf[...], NT, preferred_element_type=f32)
                hh = (silu_g * uu).astype(bf16)
                hscr[...] = hh
                nv = F - WD_VPU
                eye = lax.broadcasted_iota(jnp.int32, (nv, nv), 0) == lax.broadcasted_iota(jnp.int32, (nv, nv), 1)
                hrow = jnp.broadcast_to(hh[0:1, WD_VPU:F].astype(f32), (nv, nv))
                hcol = jnp.dot(jnp.where(eye, hrow, 0.0).astype(bf16), jnp.ones((nv, DH), bf16),
                               preferred_element_type=f32)
                hcscr[...] = hcol * (1.0 - gate)
        assert head.done() and waited == total and not q_todo and h_done

        tail_in_loop = [tail.take(max(LA - (DP - 1 - e) * kv_descs, 0)) for e in range(DP)]

        def group(g, carry):
            def kstep(c, carry):
                slot = c % NB
                wait_for(ring.at[slot], slot)

                @pl.when(c + DP < PER)
                def _():
                    issue_kv(k_hbm, g, c + DP)

                @pl.when(c + DP >= PER)
                def _():
                    issue_kv(v_hbm, g, c + DP - PER)

                s = None
                for j in range(GH):
                    t = lax.dot_general(qscr[g, :, j * DH:(j + 1) * DH], ring[slot, j], NT,
                                        preferred_element_type=f32)
                    s = t if s is None else s + t
                sscr[c] = s
                return carry

            lax.fori_loop(0, PER, kstep, 0)

            s = sscr[...] * scale
            m = jnp.max(jnp.max(s, axis=0), axis=-1, keepdims=True)
            p = jnp.exp(s - m[None])
            l = jnp.sum(jnp.sum(p, axis=0), axis=-1, keepdims=True)
            pscr[...] = p.astype(bf16)

            def vstep(c, o):
                slot = c % NB
                wait_for(ring.at[slot], slot)

                @pl.when(c + DP < PER)
                def _():
                    issue_kv(v_hbm, g, c + DP)

                @pl.when(jnp.logical_and(c + DP >= PER, g < NG - 1))
                def _():
                    issue_kv(k_hbm, g + 1, c + DP - PER)

                for e, starts in enumerate(tail_in_loop):
                    if starts:
                        @pl.when(jnp.logical_and(c + DP == PER + e, g == NG - 1))
                        def _():
                            for start in starts:
                                start()

                pc = pscr[c]
                for j in range(GH):
                    t = jnp.dot(pc, ring[slot, j], preferred_element_type=f32)
                    o = o + jnp.where(row1 == j, t, 0.0)
                return o

            o = lax.fori_loop(0, PER, vstep, jnp.zeros((GH, DH), f32))
            oscr[g] = o / l
            return carry

        lax.fori_loop(0, NG, group, 0)

        a = jnp.zeros((GH, D), f32)
        half = BATCH // 2
        for e in range(NWO):
            for part in range(2):
                upto = e * BATCH + (part + 1) * half
                tail.issue(tail.cum[min(upto + 8, len(wo_units))])
                wait_for(wobuf.at[e, pl.ds(part * 4, 4)], OS + e)
                tail.issue(tail.cum[upto] + LA)
            for j in range(8):
                h = NWO * j + e
                lhs = jnp.where(row1 == h % GH, oscr[h // GH], 0.0).astype(bf16)
                a = a + jnp.dot(lhs, wobuf[e, j], preferred_element_type=f32)
        tail.issue(ALL)
        assert tail.done()

        acc = a[0:8]
        for r in range(8, GH, 8):
            acc = acc + a[r:r + 8]
        acc = gate * acc
        row8 = lax.broadcasted_iota(jnp.int32, (8, D), 0)
        for i in range(NPIECE):
            lo, hi = WD_SPLITS[i], WD_SPLITS[i + 1]
            wait_for(wdbuf.at[pl.ds(lo, hi - lo), :], DS + i)
            if lo < WD_VPU:
                assert hi <= WD_VPU
                b = jnp.dot(hscr[:, lo:hi], wdbuf[lo:hi, :], preferred_element_type=f32)
                acc = acc + jnp.where(row8 == 0, (1.0 - gate) * b, 0.0)
            else:
                hc = hcscr[lo - WD_VPU:hi - WD_VPU, :]
                prod = wdbuf[lo:hi, :].astype(f32) * jnp.concatenate([hc] * (D // DH), axis=1)
                acc = acc + jnp.sum(prod.reshape((hi - lo) // 8, 8, D), axis=0)
        out_ref[0] = jnp.sum(acc, axis=0, keepdims=True).astype(out_ref.dtype)

    return kernel


def _compiler_params():
    kw = dict(vmem_limit_bytes=48 * 1024 * 1024)
    for name in ("disable_semaphore_checks", "disable_bounds_checks"):
        if hasattr(pltpu.CompilerParams, name):
            kw[name] = True
    return pltpu.CompilerParams(**kw)


@jax.jit
def pallas_gated_mix__sliding_block_cached__swiglu_ffn__decode_kernel(
    A_x: jax.Array,
    A_k_cache: jax.Array,
    A_v_cache: jax.Array,
    A_wq: jax.Array,
    A_wo: jax.Array,
    B_x: jax.Array,
    B_w_gate: jax.Array,
    B_w_up: jax.Array,
    B_w_down: jax.Array,
    gate_w: jax.Array,
):
    del B_x
    SK = A_k_cache.shape[2]
    W = min(4096, max(256, SK // 4))
    assert A_x.shape == (1, 1, D) and A_k_cache.shape == (1, H, SK, DH) and A_v_cache.shape == A_k_cache.shape
    assert A_wq.shape == (D, H * DH) and A_wo.shape == (H * DH, D)
    assert B_w_gate.shape == (D, F) and B_w_up.shape == (D, F) and B_w_down.shape == (F, D)
    f32, bf16 = jnp.float32, jnp.bfloat16
    per = W // BK
    hbm = pl.BlockSpec(memory_space=pl.ANY)
    return pl.pallas_call(
        _make_kernel(SK, W),
        out_shape=jax.ShapeDtypeStruct((1, 1, D), bf16),
        in_specs=[hbm] * 9,
        out_specs=pl.BlockSpec(memory_space=pltpu.VMEM),
        scratch_shapes=[
            pltpu.VMEM((1, 1, D), bf16),
            pltpu.VMEM((D,), bf16),
            pltpu.VMEM((NB, GH, BK, DH), bf16),
            pltpu.VMEM((D, H * DH), bf16),
            pltpu.VMEM((NWO, 8, DH, D), bf16),
            pltpu.VMEM((F, D), bf16),
            pltpu.VMEM((F, D), bf16),
            pltpu.VMEM((F, D), bf16),
            pltpu.VMEM((NG, GH, GW), bf16),
            pltpu.VMEM((per, GH, BK), f32),
            pltpu.VMEM((per, GH, BK), bf16),
            pltpu.VMEM((8, F), bf16),
            pltpu.VMEM((NG, GH, DH), f32),
            pltpu.VMEM((F - WD_VPU, DH), f32),
            pltpu.SemaphoreType.DMA((NB + 4 + NWO + NPIECE,)),
        ],
        compiler_params=_compiler_params(),
    )(A_x, gate_w, A_k_cache, A_v_cache, A_wq, A_wo, B_w_gate.T, B_w_up.T, B_w_down)
```

```python
import jax
import jax.numpy as jnp
from jax import lax
import jax.experimental.pallas as pl
import jax.experimental.pallas.tpu as pltpu

H, DH, D, F = 32, 128, 512, 1376
NT = (((1,), (1,)), ((), ()))

ROWS = 128
UT = 16
BATCH = 32
GH = 16
NG = H // GH
GW = GH * DH
NSUB = BATCH // GH
BK = ROWS * NSUB
DP = 3
NB = 4
LA = 192
PCHUNK = 48
NWO = 4

KV_SHIFT = 16
OFF_A = 2
OFF_B = 3

WD_T0 = 20
WD_SPLITS = (0, 896, 1152, 1272, 1336, 1376)
WD_VPU = 1152
NPIECE = len(WD_SPLITS) - 1


def _round_robin(streams):
    out = []
    for k in range(max(len(s) for s in streams)):
        out += [s[k] for s in streams if k < len(s)]
    return out


def _chop(items, n):
    return [items[i:i + n] for i in range(0, len(items), n)]


def _order128():
    streams = _chop(list(range(128)), 16)
    return _round_robin([streams[i] for i in (0, 2, 1, 3, 4, 6, 5, 7)])


def _rects(t0, t1, tb):
    out = []
    while t0 < t1:
        b, c = divmod(t0, tb)
        if c == 0 and t1 - t0 >= tb:
            nb = (t1 - t0) // tb
            out.append((8 * b, 8 * nb, 0, tb * 128))
            t0 += nb * tb
        else:
            e = min(t1, (b + 1) * tb)
            out.append((8 * b, 8, c * 128, (e - t0) * 128))
            t0 = e
    return out


def _units(nrows, ncols, off):
    tb = ncols // 128
    total = nrows // 8 * tb
    assert total % UT == 0
    units = [_rects(total - off, total, tb) + _rects(0, UT - off, tb)]
    units += [_rects(u * UT - off, (u + 1) * UT - off, tb) for u in range(1, total // UT)]
    return units


def _split_cols(rect, parts_per_unit):
    r, nr, c, nc = rect
    nt = nc // 128
    k = max(1, round(nt * parts_per_unit / UT))
    b = [round(nt * i / k) for i in range(k + 1)]
    return [(r, nr, c + 128 * b[i], 128 * (b[i + 1] - b[i])) for i in range(k)]


class _Queue:
    def __init__(self):
        self.items, self.cum, self.ptr = [], [0], 0

    def add(self, starts, ndesc=None):
        self.items.append(starts)
        self.cum.append(self.cum[-1] + (len(starts) if ndesc is None else ndesc))

    def take(self, upto):
        out = []
        while self.ptr < len(self.items) and self.cum[self.ptr + 1] <= upto:
            out += self.items[self.ptr]
            self.ptr += 1
        return out

    def issue(self, upto):
        for start in self.take(upto):
            start()

    def done(self):
        return self.ptr == len(self.items)


def _make_kernel(SK, W):
    scale = DH ** -0.5
    PER = W // BK
    S = KV_SHIFT
    ALL = 1 << 30
    f32, bf16 = jnp.float32, jnp.bfloat16
    assert W % BK == 0 and PER % NB == 0 and 2 <= DP < NB <= PER

    def kernel(x_hbm, gw_hbm, k_hbm, v_hbm, wq_hbm, wo_hbm, wg_hbm, wu_hbm, wd_hbm, out_ref,
               xbuf, gwbuf, ring, wqbuf, wobuf, wgbuf, wubuf, wdbuf,
               qscr, sscr, pscr, hscr, oscr, hcscr, sem):
        XS, QS, GS, US = NB, NB + 1, NB + 2, NB + 3
        OS = NB + 4
        DS = OS + NWO

        def wait_for(ref, s):
            pltpu.make_async_copy(ref, ref, sem.at[s]).wait()

        def start_fn(src, dst, s, prio):
            return lambda: pltpu.make_async_copy(src, dst, sem.at[s]).start(priority=prio)

        def rect_start(src, dst, rect, s, prio):
            r, nr, c, nc = rect
            return start_fn(src.at[pl.ds(r, nr), pl.ds(c, nc)], dst.at[pl.ds(r, nr), pl.ds(c, nc)], s, prio)

        def al8(v):
            return v if isinstance(v, int) else pl.multiple_of(v, 8)

        def issue_kv(src, g, c):
            slot = c % NB
            for sub in range(NSUB):
                for j in range(GH):
                    if sub == 0:
                        parts = [((c * BK + W - S) % W, 0, S), (c * BK, S, ROWS - S)]
                    else:
                        parts = [(c * BK + sub * ROWS - S, sub * ROWS, ROWS)]
                    for src_row, dst_row, n in parts:
                        pltpu.make_async_copy(
                            src.at[0, g * GH + j, pl.ds(al8(SK - W + src_row), n), :],
                            ring.at[slot, j, pl.ds(dst_row, n), :],
                            sem.at[slot]).start(priority=j % 2)

        kv_descs = GH * (NSUB + 1)

        wq_units = _units(D, H * DH, OFF_A)
        wq_order = _order128()
        assert len(wq_units) == len(wq_order)
        early = set(wq_order[:16])
        wq_units = [[p for rect in un for p in _split_cols(rect, 8 if u in early else 4)]
                    for u, un in enumerate(wq_units)]
        f_units = _units(F, D, OFF_B)
        nf = len(f_units)
        head_list = [("q", u) for u in wq_order]
        head_list += _round_robin(_chop([("g", u) for u in range(nf)], 8) + _chop([("u", u) for u in range(nf)], 8))
        info = dict(q=(wq_hbm, wqbuf, QS, wq_units, 4), g=(wg_hbm, wgbuf, GS, f_units, 32),
                    u=(wu_hbm, wubuf, US, f_units, 32))
        head = _Queue()
        for n, (kind, u) in enumerate(head_list):
            src, dst, s, units, _ = info[kind]
            starts = [rect_start(src, dst, rect, s, n % 2) for rect in units[u]]
            if n == 0:
                starts += [start_fn(x_hbm, xbuf, XS, 0), start_fn(gw_hbm, gwbuf, XS, 0)]
            head.add(starts)
        for c in range(DP):
            head.add([lambda c=c: issue_kv(k_hbm, 0, c)], kv_descs)

        tail = _Queue()
        wo_units = _units(H * DH, D, OFF_A)
        assert len(wo_units) == 128
        for n, u in enumerate(_order128()):
            starts = []
            for r, nr, c, nc in wo_units[u]:
                j, rem = divmod(r, NWO * DH)
                e, lr = divmod(rem, DH)
                assert lr + nr <= DH
                starts.append(start_fn(wo_hbm.at[pl.ds(r, nr), pl.ds(c, nc)],
                                       wobuf.at[e, j, pl.ds(lr, nr), pl.ds(c, nc)], OS + e, n % 2))
            tail.add(starts)

        def piece(r):
            return max(i for i in range(NPIECE) if WD_SPLITS[i] <= r)

        assert all(piece(r) == piece(r + nr - 1) for un in f_units for r, nr, _, _ in un)
        for u, prio in _round_robin([[(u, 0) for u in range(WD_T0)], [(u, 1) for u in range(WD_T0, nf)]]):
            tail.add([rect_start(wd_hbm, wdbuf, rect, DS + piece(rect[0]), prio) for rect in f_units[u]])

        row = lax.broadcasted_iota(jnp.int32, (GH, GW), 0)
        col = lax.broadcasted_iota(jnp.int32, (GH, GW), 1)
        diag = (col // DH) == row
        row1 = lax.broadcasted_iota(jnp.int32, (GH, DH), 0)
        total = {k: sum(1 for kind, _ in head_list if kind == k) for k in info}
        waited = {k: 0 for k in info}
        q_todo = list(range(H // 8))
        gate = silu_g = None
        h_done = False
        head.issue(LA)
        i = 0
        while i < len(head_list):
            e = i
            while e < len(head_list) and (head.cum[e + 1] - head.cum[i] <= PCHUNK or (e - i) % 2):
                e += 1
            assert head.ptr >= e
            for kind in info:
                n = sum(1 for k, _ in head_list[i:e] if k == kind)
                if n:
                    _, dst, s, _, rpu = info[kind]
                    assert (waited[kind] * rpu) % 8 == 0 and (n * rpu) % 8 == 0
                    wait_for(dst.at[pl.ds(waited[kind] * rpu, n * rpu), :], s)
                    waited[kind] += n
            head.issue(head.cum[e] + LA if e < len(head_list) else ALL)
            if i == 0:
                wait_for(xbuf, XS)
                wait_for(gwbuf, XS)
                gw = gwbuf[...].astype(f32).reshape(1, D)
                gate = jax.nn.sigmoid(jnp.sum(xbuf[0].astype(f32) * gw, axis=-1, keepdims=True))
            i = e
            if waited["q"] == total["q"]:
                for _ in range(len(q_todo) if i == len(head_list) else min(1, len(q_todo))):
                    g8 = q_todo.pop(0)
                    g, lo = divmod(g8 * 8 * DH, GW)
                    q = jnp.dot(jnp.broadcast_to(xbuf[0], (GH, D)), wqbuf[:, g8 * 8 * DH:(g8 + 1) * 8 * DH],
                                preferred_element_type=f32)
                    qscr[g, :, lo:lo + 8 * DH] = jnp.where(diag[:, lo:lo + 8 * DH], q, 0.0).astype(bf16)
            if silu_g is None and waited["g"] == total["g"]:
                gg = lax.dot_general(jnp.broadcast_to(xbuf[0], (8, D)), wgbuf[...], NT, preferred_element_type=f32)
                silu_g = gg * jax.nn.sigmoid(gg)
            if not h_done and silu_g is not None and waited["u"] == total["u"]:
                h_done = True
                uu = lax.dot_general(jnp.broadcast_to(xbuf[0], (8, D)), wubuf[...], NT, preferred_element_type=f32)
                hh = (silu_g * uu).astype(bf16)
                hscr[...] = hh
                nv = F - WD_VPU
                eye = lax.broadcasted_iota(jnp.int32, (nv, nv), 0) == lax.broadcasted_iota(jnp.int32, (nv, nv), 1)
                hrow = jnp.broadcast_to(hh[0:1, WD_VPU:F].astype(f32), (nv, nv))
                hcol = jnp.dot(jnp.where(eye, hrow, 0.0).astype(bf16), jnp.ones((nv, DH), bf16),
                               preferred_element_type=f32)
                hcscr[...] = hcol * (1.0 - gate)
        assert head.done() and waited == total and not q_todo and h_done

        tail_in_loop = [tail.take(max(LA - (DP - 1 - e) * kv_descs, 0)) for e in range(DP)]

        def group(g, carry):
            def kstep(c, carry):
                slot = c % NB
                wait_for(ring.at[slot], slot)

                @pl.when(c + DP < PER)
                def _():
                    issue_kv(k_hbm, g, c + DP)

                @pl.when(c + DP >= PER)
                def _():
                    issue_kv(v_hbm, g, c + DP - PER)

                s = None
                for j in range(GH):
                    t = lax.dot_general(qscr[g, :, j * DH:(j + 1) * DH], ring[slot, j], NT,
                                        preferred_element_type=f32)
                    s = t if s is None else s + t
                sscr[c] = s
                return carry

            lax.fori_loop(0, PER, kstep, 0)

            s = sscr[...] * scale
            m = jnp.max(jnp.max(s, axis=0), axis=-1, keepdims=True)
            p = jnp.exp(s - m[None])
            l = jnp.sum(jnp.sum(p, axis=0), axis=-1, keepdims=True)
            pscr[...] = p.astype(bf16)

            def vstep(c, o):
                slot = c % NB
                wait_for(ring.at[slot], slot)

                @pl.when(c + DP < PER)
                def _():
                    issue_kv(v_hbm, g, c + DP)

                @pl.when(jnp.logical_and(c + DP >= PER, g < NG - 1))
                def _():
                    issue_kv(k_hbm, g + 1, c + DP - PER)

                for e, starts in enumerate(tail_in_loop):
                    if starts:
                        @pl.when(jnp.logical_and(c + DP == PER + e, g == NG - 1))
                        def _():
                            for start in starts:
                                start()

                pc = pscr[c]
                for j in range(GH):
                    t = jnp.dot(pc, ring[slot, j], preferred_element_type=f32)
                    o = o + jnp.where(row1 == j, t, 0.0)
                return o

            o = lax.fori_loop(0, PER, vstep, jnp.zeros((GH, DH), f32))
            oscr[g] = o / l
            return carry

        lax.fori_loop(0, NG, group, 0)

        a = jnp.zeros((GH, D), f32)
        half = BATCH // 2
        for e in range(NWO):
            for part in range(2):
                upto = e * BATCH + (part + 1) * half
                tail.issue(tail.cum[min(upto + 8, len(wo_units))])
                wait_for(wobuf.at[e, pl.ds(part * 4, 4)], OS + e)
                tail.issue(tail.cum[upto] + LA)
            for j in range(8):
                h = NWO * j + e
                lhs = jnp.where(row1 == h % GH, oscr[h // GH], 0.0).astype(bf16)
                a = a + jnp.dot(lhs, wobuf[e, j], preferred_element_type=f32)
        tail.issue(ALL)
        assert tail.done()

        acc = a[0:8]
        for r in range(8, GH, 8):
            acc = acc + a[r:r + 8]
        acc = gate * acc
        row8 = lax.broadcasted_iota(jnp.int32, (8, D), 0)
        for i in range(NPIECE):
            lo, hi = WD_SPLITS[i], WD_SPLITS[i + 1]
            wait_for(wdbuf.at[pl.ds(lo, hi - lo), :], DS + i)
            if lo < WD_VPU:
                assert hi <= WD_VPU
                b = jnp.dot(hscr[:, lo:hi], wdbuf[lo:hi, :], preferred_element_type=f32)
                acc = acc + jnp.where(row8 == 0, (1.0 - gate) * b, 0.0)
            else:
                hc = hcscr[lo - WD_VPU:hi - WD_VPU, :]
                prod = wdbuf[lo:hi, :].astype(f32) * jnp.concatenate([hc] * (D // DH), axis=1)
                acc = acc + jnp.sum(prod.reshape((hi - lo) // 8, 8, D), axis=0)
        out_ref[0] = jnp.sum(acc, axis=0, keepdims=True).astype(out_ref.dtype)

    return kernel


def _compiler_params():
    kw = dict(vmem_limit_bytes=48 * 1024 * 1024)
    if hasattr(pltpu.CompilerParams, "disable_semaphore_checks"):
        kw["disable_semaphore_checks"] = True
    return pltpu.CompilerParams(**kw)


@jax.jit
def pallas_gated_mix__sliding_block_cached__swiglu_ffn__decode_kernel(
    A_x: jax.Array,
    A_k_cache: jax.Array,
    A_v_cache: jax.Array,
    A_wq: jax.Array,
    A_wo: jax.Array,
    B_x: jax.Array,
    B_w_gate: jax.Array,
    B_w_up: jax.Array,
    B_w_down: jax.Array,
    gate_w: jax.Array,
):
    del B_x
    SK = A_k_cache.shape[2]
    W = min(4096, max(256, SK // 4))
    assert A_x.shape == (1, 1, D) and A_k_cache.shape == (1, H, SK, DH) and A_v_cache.shape == A_k_cache.shape
    assert A_wq.shape == (D, H * DH) and A_wo.shape == (H * DH, D)
    assert B_w_gate.shape == (D, F) and B_w_up.shape == (D, F) and B_w_down.shape == (F, D)
    f32, bf16 = jnp.float32, jnp.bfloat16
    per = W // BK
    hbm = pl.BlockSpec(memory_space=pl.ANY)
    return pl.pallas_call(
        _make_kernel(SK, W),
        out_shape=jax.ShapeDtypeStruct((1, 1, D), bf16),
        in_specs=[hbm] * 9,
        out_specs=pl.BlockSpec(memory_space=pltpu.VMEM),
        scratch_shapes=[
            pltpu.VMEM((1, 1, D), bf16),
            pltpu.VMEM((D,), bf16),
            pltpu.VMEM((NB, GH, BK, DH), bf16),
            pltpu.VMEM((D, H * DH), bf16),
            pltpu.VMEM((NWO, 8, DH, D), bf16),
            pltpu.VMEM((F, D), bf16),
            pltpu.VMEM((F, D), bf16),
            pltpu.VMEM((F, D), bf16),
            pltpu.VMEM((NG, GH, GW), bf16),
            pltpu.VMEM((per, GH, BK), f32),
            pltpu.VMEM((per, GH, BK), bf16),
            pltpu.VMEM((8, F), bf16),
            pltpu.VMEM((NG, GH, DH), f32),
            pltpu.VMEM((F - WD_VPU, DH), f32),
            pltpu.SemaphoreType.DMA((NB + 4 + NWO + NPIECE,)),
        ],
        compiler_params=_compiler_params(),
    )(A_x, gate_w, A_k_cache, A_v_cache, A_wq, A_wo, B_w_gate.T, B_w_up.T, B_w_down)
```

```python
import jax
import jax.numpy as jnp
from jax import lax
import jax.experimental.pallas as pl
import jax.experimental.pallas.tpu as pltpu

H, DH, D, F = 32, 128, 512, 1376
NT = (((1,), (1,)), ((), ()))

ROWS = 128
UT = 16
BATCH = 32
GH = 16
NG = H // GH
GW = GH * DH
NSUB = BATCH // GH
BK = ROWS * NSUB
DP = 3
NB = 4
LA = 192
PCHUNK = 48
NWO = 4

KV_SHIFT = 16
OFF_A = 2
OFF_B = 3

WD_T0 = 20
WD_SPLITS = (0, 896, 1152, 1272, 1336, 1376)
WD_VPU = 1152
NPIECE = len(WD_SPLITS) - 1


def _round_robin(streams):
    out = []
    for k in range(max(len(s) for s in streams)):
        out += [s[k] for s in streams if k < len(s)]
    return out


def _chop(items, n):
    return [items[i:i + n] for i in range(0, len(items), n)]


def _order128():
    streams = _chop(list(range(128)), 16)
    return _round_robin([streams[i] for i in (0, 2, 1, 3, 4, 6, 5, 7)])


def _rects(t0, t1, tb):
    out = []
    while t0 < t1:
        b, c = divmod(t0, tb)
        if c == 0 and t1 - t0 >= tb:
            nb = (t1 - t0) // tb
            out.append((8 * b, 8 * nb, 0, tb * 128))
            t0 += nb * tb
        else:
            e = min(t1, (b + 1) * tb)
            out.append((8 * b, 8, c * 128, (e - t0) * 128))
            t0 = e
    return out


def _units(nrows, ncols, off):
    tb = ncols // 128
    total = nrows // 8 * tb
    assert total % UT == 0
    units = [_rects(total - off, total, tb) + _rects(0, UT - off, tb)]
    units += [_rects(u * UT - off, (u + 1) * UT - off, tb) for u in range(1, total // UT)]
    return units


def _split_cols(rect, parts_per_unit):
    r, nr, c, nc = rect
    nt = nc // 128
    k = max(1, round(nt * parts_per_unit / UT))
    b = [round(nt * i / k) for i in range(k + 1)]
    return [(r, nr, c + 128 * b[i], 128 * (b[i + 1] - b[i])) for i in range(k)]


class _Queue:
    def __init__(self):
        self.items, self.cum, self.ptr = [], [0], 0

    def add(self, starts, ndesc=None):
        self.items.append(starts)
        self.cum.append(self.cum[-1] + (len(starts) if ndesc is None else ndesc))

    def take(self, upto):
        out = []
        while self.ptr < len(self.items) and self.cum[self.ptr + 1] <= upto:
            out += self.items[self.ptr]
            self.ptr += 1
        return out

    def issue(self, upto):
        for start in self.take(upto):
            start()

    def done(self):
        return self.ptr == len(self.items)


def _make_kernel(SK, W):
    scale = DH ** -0.5
    PER = W // BK
    S = KV_SHIFT
    ALL = 1 << 30
    f32, bf16 = jnp.float32, jnp.bfloat16
    assert W % BK == 0 and PER % NB == 0 and 2 <= DP < NB <= PER

    def kernel(x_hbm, gw_hbm, k_hbm, v_hbm, wq_hbm, wo_hbm, wg_hbm, wu_hbm, wd_hbm, out_ref,
               xbuf, gwbuf, ring, wqbuf, wobuf, wgbuf, wubuf, wdbuf,
               qscr, sscr, pscr, hscr, oscr, hcscr, sem):
        XS, QS, GS, US = NB, NB + 1, NB + 2, NB + 3
        OS = NB + 4
        DS = OS + NWO

        def wait_for(ref, s):
            pltpu.make_async_copy(ref, ref, sem.at[s]).wait()

        class Copy:
            def __init__(self, src, dst, s, prio):
                self.src, self.dst, self.s, self.prio = src, dst, s, prio

            def __call__(self):
                pltpu.make_async_copy(self.src, self.dst, sem.at[self.s]).start(priority=self.prio)

            def wait(self):
                pltpu.make_async_copy(self.src, self.dst, sem.at[self.s]).wait()

        def rect_copy(src, dst, rect, s, prio):
            r, nr, c, nc = rect
            return Copy(src.at[pl.ds(r, nr), pl.ds(c, nc)], dst.at[pl.ds(r, nr), pl.ds(c, nc)], s, prio)

        def wait_all(copies):
            for cp in sorted(copies, key=lambda cp: cp.s):
                cp.wait()

        def al8(v):
            return v if isinstance(v, int) else pl.multiple_of(v, 8)

        def issue_kv(src, g, c):
            slot = c % NB
            for sub in range(NSUB):
                for j in range(GH):
                    if sub == 0:
                        parts = [((c * BK + W - S) % W, 0, S), (c * BK, S, ROWS - S)]
                    else:
                        parts = [(c * BK + sub * ROWS - S, sub * ROWS, ROWS)]
                    for src_row, dst_row, n in parts:
                        pltpu.make_async_copy(
                            src.at[0, g * GH + j, pl.ds(al8(SK - W + src_row), n), :],
                            ring.at[slot, j, pl.ds(dst_row, n), :],
                            sem.at[slot]).start(priority=j % 2)

        kv_descs = GH * (NSUB + 1)

        wq_units = _units(D, H * DH, OFF_A)
        wq_order = _order128()
        assert len(wq_units) == len(wq_order)
        early = set(wq_order[:16])
        wq_units = [[p for rect in un for p in _split_cols(rect, 8 if u in early else 4)]
                    for u, un in enumerate(wq_units)]
        f_units = _units(F, D, OFF_B)
        nf = len(f_units)
        head_list = [("q", u) for u in wq_order]
        head_list += _round_robin(_chop([("g", u) for u in range(nf)], 8) + _chop([("u", u) for u in range(nf)], 8))
        info = dict(q=(wq_hbm, wqbuf, QS, wq_units), g=(wg_hbm, wgbuf, GS, f_units), u=(wu_hbm, wubuf, US, f_units))
        head = _Queue()
        for n, (kind, u) in enumerate(head_list):
            src, dst, s, units = info[kind]
            starts = [rect_copy(src, dst, rect, s, n % 2) for rect in units[u]]
            if n == 0:
                starts += [Copy(x_hbm, xbuf, XS, 0), Copy(gw_hbm, gwbuf, XS, 0)]
            head.add(starts)
        for c in range(DP):
            head.add([lambda c=c: issue_kv(k_hbm, 0, c)], kv_descs)

        tail = _Queue()
        wo_units = _units(H * DH, D, OFF_A)
        assert len(wo_units) == 128
        for n, u in enumerate(_order128()):
            starts = []
            for r, nr, c, nc in wo_units[u]:
                j, rem = divmod(r, NWO * DH)
                e, lr = divmod(rem, DH)
                assert lr + nr <= DH
                starts.append(Copy(wo_hbm.at[pl.ds(r, nr), pl.ds(c, nc)],
                                   wobuf.at[e, j, pl.ds(lr, nr), pl.ds(c, nc)], OS + e, n % 2))
            tail.add(starts)

        def piece(r):
            return max(i for i in range(NPIECE) if WD_SPLITS[i] <= r)

        assert all(piece(r) == piece(r + nr - 1) for un in f_units for r, nr, _, _ in un)
        for u, prio in _round_robin([[(u, 0) for u in range(WD_T0)], [(u, 1) for u in range(WD_T0, nf)]]):
            tail.add([rect_copy(wd_hbm, wdbuf, rect, DS + piece(rect[0]), prio) for rect in f_units[u]])

        row = lax.broadcasted_iota(jnp.int32, (GH, GW), 0)
        col = lax.broadcasted_iota(jnp.int32, (GH, GW), 1)
        diag = (col // DH) == row
        row1 = lax.broadcasted_iota(jnp.int32, (GH, DH), 0)
        total = {k: sum(1 for kind, _ in head_list if kind == k) for k in info}
        waited = {k: 0 for k in info}
        q_todo = list(range(H // 8))
        gate = silu_g = None
        h_done = False
        head.issue(LA)
        i = 0
        while i < len(head_list):
            e = i
            while e < len(head_list) and (head.cum[e + 1] - head.cum[i] <= PCHUNK or (e - i) % 2):
                e += 1
            assert head.ptr >= e
            wait_all([cp for item in head.items[i:e] for cp in item])
            for kind, _ in head_list[i:e]:
                waited[kind] += 1
            head.issue(head.cum[e] + LA if e < len(head_list) else ALL)
            if i == 0:
                gw = gwbuf[...].astype(f32).reshape(1, D)
                gate = jax.nn.sigmoid(jnp.sum(xbuf[0].astype(f32) * gw, axis=-1, keepdims=True))
            i = e
            if waited["q"] == total["q"]:
                for _ in range(len(q_todo) if i == len(head_list) else min(1, len(q_todo))):
                    g8 = q_todo.pop(0)
                    g, lo = divmod(g8 * 8 * DH, GW)
                    q = jnp.dot(jnp.broadcast_to(xbuf[0], (GH, D)), wqbuf[:, g8 * 8 * DH:(g8 + 1) * 8 * DH],
                                preferred_element_type=f32)
                    qscr[g, :, lo:lo + 8 * DH] = jnp.where(diag[:, lo:lo + 8 * DH], q, 0.0).astype(bf16)
            if silu_g is None and waited["g"] == total["g"]:
                gg = lax.dot_general(jnp.broadcast_to(xbuf[0], (8, D)), wgbuf[...], NT, preferred_element_type=f32)
                silu_g = gg * jax.nn.sigmoid(gg)
            if not h_done and silu_g is not None and waited["u"] == total["u"]:
                h_done = True
                uu = lax.dot_general(jnp.broadcast_to(xbuf[0], (8, D)), wubuf[...], NT, preferred_element_type=f32)
                hh = (silu_g * uu).astype(bf16)
                hscr[...] = hh
                nv = F - WD_VPU
                eye = lax.broadcasted_iota(jnp.int32, (nv, nv), 0) == lax.broadcasted_iota(jnp.int32, (nv, nv), 1)
                hrow = jnp.broadcast_to(hh[0:1, WD_VPU:F].astype(f32), (nv, nv))
                hcol = jnp.dot(jnp.where(eye, hrow, 0.0).astype(bf16), jnp.ones((nv, DH), bf16),
                               preferred_element_type=f32)
                hcscr[...] = hcol * (1.0 - gate)
        assert head.done() and waited == total and not q_todo and h_done

        tail_in_loop = [tail.take(max(LA - (DP - 1 - e) * kv_descs, 0)) for e in range(DP)]

        def group(g, carry):
            def kstep(c, carry):
                slot = c % NB
                wait_for(ring.at[slot], slot)

                @pl.when(c + DP < PER)
                def _():
                    issue_kv(k_hbm, g, c + DP)

                @pl.when(c + DP >= PER)
                def _():
                    issue_kv(v_hbm, g, c + DP - PER)

                s = None
                for j in range(GH):
                    t = lax.dot_general(qscr[g, :, j * DH:(j + 1) * DH], ring[slot, j], NT,
                                        preferred_element_type=f32)
                    s = t if s is None else s + t
                sscr[c] = s
                return carry

            lax.fori_loop(0, PER, kstep, 0)

            s = sscr[...] * scale
            m = jnp.max(jnp.max(s, axis=0), axis=-1, keepdims=True)
            p = jnp.exp(s - m[None])
            l = jnp.sum(jnp.sum(p, axis=0), axis=-1, keepdims=True)
            pscr[...] = p.astype(bf16)

            def vstep(c, o):
                slot = c % NB
                wait_for(ring.at[slot], slot)

                @pl.when(c + DP < PER)
                def _():
                    issue_kv(v_hbm, g, c + DP)

                @pl.when(jnp.logical_and(c + DP >= PER, g < NG - 1))
                def _():
                    issue_kv(k_hbm, g + 1, c + DP - PER)

                for e, starts in enumerate(tail_in_loop):
                    if starts:
                        @pl.when(jnp.logical_and(c + DP == PER + e, g == NG - 1))
                        def _():
                            for start in starts:
                                start()

                pc = pscr[c]
                for j in range(GH):
                    t = jnp.dot(pc, ring[slot, j], preferred_element_type=f32)
                    o = o + jnp.where(row1 == j, t, 0.0)
                return o

            o = lax.fori_loop(0, PER, vstep, jnp.zeros((GH, DH), f32))
            oscr[g] = o / l
            return carry

        lax.fori_loop(0, NG, group, 0)

        a = jnp.zeros((GH, D), f32)
        half = BATCH // 2
        for e in range(NWO):
            mine = [(n, cp) for n, item in enumerate(tail.items) for cp in item if cp.s == OS + e]
            for part in range(2):
                upto = e * BATCH + (part + 1) * half
                some = [(n, cp) for n, cp in mine if (n < e * BATCH + half) == (part == 0)]
                tail.issue(tail.cum[max(n for n, _ in some) + 1])
                wait_all([cp for _, cp in some])
                tail.issue(tail.cum[upto] + LA)
            for j in range(8):
                h = NWO * j + e
                lhs = jnp.where(row1 == h % GH, oscr[h // GH], 0.0).astype(bf16)
                a = a + jnp.dot(lhs, wobuf[e, j], preferred_element_type=f32)
        tail.issue(ALL)
        assert tail.done()

        acc = a[0:8]
        for r in range(8, GH, 8):
            acc = acc + a[r:r + 8]
        acc = gate * acc
        row8 = lax.broadcasted_iota(jnp.int32, (8, D), 0)
        for i in range(NPIECE):
            lo, hi = WD_SPLITS[i], WD_SPLITS[i + 1]
            wait_for(wdbuf.at[pl.ds(lo, hi - lo), :], DS + i)
            if lo < WD_VPU:
                assert hi <= WD_VPU
                b = jnp.dot(hscr[:, lo:hi], wdbuf[lo:hi, :], preferred_element_type=f32)
                acc = acc + jnp.where(row8 == 0, (1.0 - gate) * b, 0.0)
            else:
                hc = hcscr[lo - WD_VPU:hi - WD_VPU, :]
                prod = wdbuf[lo:hi, :].astype(f32) * jnp.concatenate([hc] * (D // DH), axis=1)
                acc = acc + jnp.sum(prod.reshape((hi - lo) // 8, 8, D), axis=0)
        out_ref[0] = jnp.sum(acc, axis=0, keepdims=True).astype(out_ref.dtype)

    return kernel


def _compiler_params():
    kw = dict(vmem_limit_bytes=48 * 1024 * 1024)
    if hasattr(pltpu.CompilerParams, "disable_semaphore_checks"):
        kw["disable_semaphore_checks"] = True
    return pltpu.CompilerParams(**kw)


@jax.jit
def pallas_gated_mix__sliding_block_cached__swiglu_ffn__decode_kernel(
    A_x: jax.Array,
    A_k_cache: jax.Array,
    A_v_cache: jax.Array,
    A_wq: jax.Array,
    A_wo: jax.Array,
    B_x: jax.Array,
    B_w_gate: jax.Array,
    B_w_up: jax.Array,
    B_w_down: jax.Array,
    gate_w: jax.Array,
):
    del B_x
    SK = A_k_cache.shape[2]
    W = min(4096, max(256, SK // 4))
    assert A_x.shape == (1, 1, D) and A_k_cache.shape == (1, H, SK, DH) and A_v_cache.shape == A_k_cache.shape
    assert A_wq.shape == (D, H * DH) and A_wo.shape == (H * DH, D)
    assert B_w_gate.shape == (D, F) and B_w_up.shape == (D, F) and B_w_down.shape == (F, D)
    f32, bf16 = jnp.float32, jnp.bfloat16
    per = W // BK
    hbm = pl.BlockSpec(memory_space=pl.ANY)
    return pl.pallas_call(
        _make_kernel(SK, W),
        out_shape=jax.ShapeDtypeStruct((1, 1, D), bf16),
        in_specs=[hbm] * 9,
        out_specs=pl.BlockSpec(memory_space=pltpu.VMEM),
        scratch_shapes=[
            pltpu.VMEM((1, 1, D), bf16),
            pltpu.VMEM((D,), bf16),
            pltpu.VMEM((NB, GH, BK, DH), bf16),
            pltpu.VMEM((D, H * DH), bf16),
            pltpu.VMEM((NWO, 8, DH, D), bf16),
            pltpu.VMEM((F, D), bf16),
            pltpu.VMEM((F, D), bf16),
            pltpu.VMEM((F, D), bf16),
            pltpu.VMEM((NG, GH, GW), bf16),
            pltpu.VMEM((per, GH, BK), f32),
            pltpu.VMEM((per, GH, BK), bf16),
            pltpu.VMEM((8, F), bf16),
            pltpu.VMEM((NG, GH, DH), f32),
            pltpu.VMEM((F - WD_VPU, DH), f32),
            pltpu.SemaphoreType.DMA((NB + 4 + NWO + NPIECE,)),
        ],
        compiler_params=_compiler_params(),
    )(A_x, gate_w, A_k_cache, A_v_cache, A_wq, A_wo, B_w_gate.T, B_w_up.T, B_w_down)
```
